```python
import jax
import jax.numpy as jnp

def _softmax(x, axis=-1):
    return jax.nn.softmax(x, axis=axis)

def _gelu(x):
    return jax.nn.gelu(x, approximate=True)

def _silu(x):
    return jax.nn.silu(x)

def _sigmoid(x):
    return jax.nn.sigmoid(x)

def _layernorm(x, axis=-1, eps=1e-05):
    m = jnp.mean(x, axis=axis, keepdims=True)
    v = jnp.var(x, axis=axis, keepdims=True)
    return (x - m) / jnp.sqrt(v + eps)

def _scatter_add(tgt, idx, src, axis=0):
    return tgt.at[idx].add(src)

def _segment_sum(src, seg, n):
    return jax.ops.segment_sum(src, seg, n)

class _Rng:

    def __init__(self, key):
        self._k = key

    def _next(self):
        self._k, sub = jax.random.split(self._k)
        return sub

    def normal(self, shape):
        return jax.random.normal(self._next(), shape, dtype=jnp.bfloat16)

    def randint(self, lo, hi, shape):
        return jax.random.randint(self._next(), shape, lo, hi, dtype=jnp.int32)

    def uniform(self, shape, lo=0.0, hi=1.0):
        return jax.random.uniform(self._next(), shape, jnp.bfloat16, lo, hi)

    def permutation(self, n):
        return jax.random.permutation(self._next(), n)
kernel_name = 'adaLN_cond__sliding_local_dilated__moe_arch_mod__prompt'

def setup_inputs():
    _rng = _Rng(jax.random.key(int.from_bytes(__import__("os").urandom(4), "little")))
    _w = lambda a: (lambda t: t.astype(jnp.bfloat16) if jnp.issubdtype(t.dtype, jnp.floating) else t)(jnp.asarray(a))

    def _A_setup():
        B, S, D = (1, 2048, 640)
        return {'x': _w((lambda *s: _rng.normal(s) * 0.05)(B, S, D)), 'wqkv': _w((lambda *s: _rng.normal(s) * 0.05)(D, 3 * D)), 'wo': _w((lambda *s: _rng.normal(s) * 0.05)(D, D))}
    _A_in = _A_setup()

    def _B_setup():
        B, S, D, F, C = (1, 2048, 640, 1728, 1)
        return {'x': _w((lambda *s: _rng.normal(s) * 0.05)(B, S, D)), 'w_r': _w((lambda *s: _rng.normal(s) * 0.05)(D)), 'w_gate': _w((lambda *s: _rng.normal(s) * 0.05)(D, F)), 'w_up': _w((lambda *s: _rng.normal(s) * 0.05)(D, F)), 'w_down': _w((lambda *s: _rng.normal(s) * 0.05)(F, D))}
    _B_in = _B_setup()
    return {'A_x': _A_in['x'], 'A_wqkv': _A_in['wqkv'], 'A_wo': _A_in['wo'], 'B_x': _B_in['x'], 'B_w_r': _B_in['w_r'], 'B_w_gate': _B_in['w_gate'], 'B_w_up': _B_in['w_up'], 'B_w_down': _B_in['w_down'], 'c': _w((lambda *s: _rng.normal(s) * 0.05)(1, 640)), 'w_mod': _w((lambda *s: _rng.normal(s) * 0.05)(640, 6 * 640) * 640 ** (-0.5))}

def reference(A_x, A_wqkv, A_wo, B_x, B_w_r, B_w_gate, B_w_up, B_w_down, c, w_mod):

    def _A_ref(x, wqkv, wo):
        B, S, D = x.shape
        H = 32
        Dh = D // H
        W, dil = (8, 2)
        qkv = (lambda x, *d: x.transpose(*d))((x @ wqkv).reshape(B, S, 3, H, Dh), 2, 0, 3, 1, 4)
        q, k, v = (qkv[0], qkv[1], qkv[2])
        scale = Dh ** (-0.5)
        pos = jnp.arange(S)
        off = jnp.arange(W) * dil
        idx = pos[:, None] - off[None, :]
        mask = idx >= 0
        idx_c = jnp.where(mask, idx, 0).reshape(-1)
        kg = k[:, :, idx_c, :].reshape(B, H, S, W, Dh)
        vg = v[:, :, idx_c, :].reshape(B, H, S, W, Dh)
        logits = jnp.einsum('bhsd,bhswd->bhsw', q, kg) * scale
        logits = jnp.where(mask[None, None, :, :], logits, -1000000000.0)
        attn = _softmax(logits, axis=-1)
        o = jnp.einsum('bhsw,bhswd->bhsd', attn, vg)
        return (lambda x, *d: x.transpose(*d))(o, 0, 2, 1, 3).reshape(B, S, D) @ wo

    def _B_ref(x, w_r, w_gate, w_up, w_down):
        B, S, D = x.shape
        C = 1
        r = x @ w_r
        idx = jnp.argsort(-r, axis=-1)[:, :C]
        idx_e = jnp.repeat(idx.reshape(B, C, 1), D, axis=2)
        x_sel = jnp.take_along_axis(x, idx_e, axis=1)
        g = _silu(x_sel @ w_gate)
        u = x_sel @ w_up
        y = g * u @ w_down
        r_sel = _sigmoid(jnp.take_along_axis(r, idx, axis=1))
        y = y * r_sel.reshape(B, C, 1)
        b_off = (jnp.arange(B) * S).reshape(B, 1)
        flat_idx = (idx + b_off).reshape(B * C)
        zero = (x * 0.0).reshape(B * S, D)
        upd = _scatter_add(zero, flat_idx, y.reshape(B * C, D), axis=0)
        return x + upd.reshape(B, S, D)
    x = A_x
    mod = (_silu(c) @ w_mod).reshape(c.shape[0], 6, 1, -1)
    sa, ca, ga, sb, cb, gb = (mod[:, 0].copy(), mod[:, 1].copy(), mod[:, 2].copy(), mod[:, 3].copy(), mod[:, 4].copy(), mod[:, 5].copy())
    h = _layernorm(x, axis=-1) * (1 + ca) + sa
    x = x + ga * _A_ref(h, A_wqkv, A_wo)
    h = _layernorm(x, axis=-1) * (1 + cb) + sb
    x = x + gb * _B_ref(h, B_w_r, B_w_gate, B_w_up, B_w_down)
    return x
```

```python
import functools
import math

import jax
import jax.numpy as jnp
from jax import lax
import jax.experimental.pallas as pl
import jax.experimental.pallas.tpu as pltpu

S = 2048
D = 640
H = 32
DH = 20
WIN = 8
DIL = 2
F = 1728
NJ = D // 128
TM = 256
NT = S // TM
HALO = 16
RG = 8
EPS = 1e-5
LOG2E = math.log2(math.e)
QSCALE = (DH ** -0.5) * LOG2E
NEG = -1000000000.0 * LOG2E
f32 = jnp.float32
bf16 = jnp.bfloat16


def _kernel(x_hbm, wqkv_hbm, wo_hbm, wr_hbm, wg_hbm, wu_hbm, wd_hbm, c_hbm, wmod_hbm,
            out_hbm,
            x_v, wqkv_raw, wqkv_p, wo_raw, wo_f, wo_p, wg_v, wu_v, wd_v, wmod_v, c_v, wr_v,
            mod_v, h_v, qa, qb, ka, kb, va, vb, oa, ob, x1_v, h2_v, out_v, best_v, besti_v,
            sems, osems):
    def cp(src, dst, i):
        return pltpu.make_async_copy(src, dst, sems.at[i])

    c_cp = cp(c_hbm, c_v, 0)
    wr_cp = cp(wr_hbm, wr_v, 1)
    x0_cp = cp(x_hbm.at[pl.ds(0, TM)], x_v.at[pl.ds(0, TM)], 2)
    wm0_cp = cp(wmod_hbm.at[:, pl.ds(0, 2 * D)], wmod_v.at[:, pl.ds(0, 2 * D)], 3)
    wqkv_cp = cp(wqkv_hbm, wqkv_raw, 4)
    xr_cp = cp(x_hbm.at[pl.ds(TM, S - TM)], x_v.at[pl.ds(TM, S - TM)], 5)
    wo_cp = cp(wo_hbm, wo_raw, 6)
    wm1_cp = cp(wmod_hbm.at[:, pl.ds(2 * D, 4 * D)], wmod_v.at[:, pl.ds(2 * D, 4 * D)], 7)
    wg_cp = cp(wg_hbm, wg_v, 8)
    wu_cp = cp(wu_hbm, wu_v, 9)
    wd_cp = cp(wd_hbm, wd_v, 10)
    for d in (c_cp, x0_cp, wm0_cp, wqkv_cp, wr_cp, xr_cp, wo_cp, wm1_cp, wg_cp, wu_cp, wd_cp):
        d.start()

    def mod_part(lo, hi):
        c = c_v[...].astype(f32)
        sc = (c * jax.nn.sigmoid(c)).astype(bf16)
        sc = jnp.broadcast_to(sc, (16, D))
        m = jnp.dot(sc, wmod_v[:, lo:hi], preferred_element_type=f32)
        mod_v[:, lo:hi] = m[:8].astype(bf16).astype(f32)

    def permute_wqkv():
        lane = lax.broadcasted_iota(jnp.int32, (8, 128), 1)
        quad = lane // 4
        for t in range(3):
            for j in range(NJ):
                idx = 4 * ((5 * (lane % 32) + j) % 32) + lane // 32
                src_blk = ((j + 5 * 32 - quad) * 3) % 5
                masks = [src_blk == i for i in range(1, NJ)]
                for r in range(D // 16):
                    srcs = [pltpu.bitcast(wqkv_raw[r * 16:(r + 1) * 16,
                                                   t * D + i * 128:t * D + (i + 1) * 128], jnp.uint32)
                            for i in range(NJ)]
                    m = srcs[0]
                    for i in range(1, NJ):
                        m = jnp.where(masks[i - 1], srcs[i], m)
                    y = jnp.take_along_axis(m, idx, axis=1)
                    wqkv_p[r * 16:(r + 1) * 16, t * D + j * 128:t * D + (j + 1) * 128] = (
                        pltpu.bitcast(y, bf16))

    def permute_wo():
        for n in range(NJ):
            wo_f[n] = wo_raw[:, n * 128:(n + 1) * 128].astype(f32)
        for n in range(NJ):
            for j in range(NJ):
                for dd in range(4):
                    rows = wo_f[n, pl.ds(4 * j + dd, H, stride=DH), :]
                    wo_p[j * 128 + dd * 32:j * 128 + (dd + 1) * 32, n * 128:(n + 1) * 128] = rows.astype(bf16)

    def ln_rows(xf):
        m = jnp.sum(xf, axis=-1, keepdims=True) * (1.0 / D)
        xc = xf - m
        v = jnp.sum(xc * xc, axis=-1, keepdims=True) * (1.0 / D)
        return xc * lax.rsqrt(v + EPS)

    def ln1(row0):
        xf = x_v[pl.ds(row0, TM), :].astype(f32)
        n = ln_rows(xf)
        sa = mod_v[0:1, 0:D]
        ca = mod_v[0:1, D:2 * D]
        h_v[...] = (n * (1.0 + ca) + sa).astype(bf16)

    def qkv(q_r, k_r, v_r):
        res = jnp.dot(h_v[...], wqkv_p[...], preferred_element_type=f32)
        for j in range(NJ):
            q_r[j] = res[:, j * 128:(j + 1) * 128] * QSCALE
            k_r[j, HALO:HALO + TM, :] = res[:, D + j * 128:D + (j + 1) * 128]
            v_r[j, HALO:HALO + TM, :] = res[:, 2 * D + j * 128:2 * D + (j + 1) * 128]

    def halo(k_src, v_src, k_dst, v_dst):
        for j in range(NJ):
            k_dst[j, 0:HALO, :] = k_src[j, TM:TM + HALO, :]
            v_dst[j, 0:HALO, :] = v_src[j, TM:TM + HALO, :]

    def attention(row0, q_r, k_r, v_r, o_r):
        ng = TM // RG
        st1 = {}
        st2 = {}
        outs = {}

        def stage1(g):
            r0 = g * RG
            q = [q_r[j, pl.ds(r0, RG), :] for j in range(NJ)]
            ps = []
            for w in range(WIN):
                off = HALO + r0 - DIL * w
                p = q[0] * k_r[0, pl.ds(off, RG), :]
                for j in range(1, NJ):
                    p = p + q[j] * k_r[j, pl.ds(off, RG), :]
                ps.append((p, pltpu.roll(p, 64, 1)))
            st1[g] = ps

        def stage2(g):
            ps = []
            for (p, pr) in st1.pop(g):
                p = p + pr
                ps.append((p, pltpu.roll(p, 32, 1)))
            st2[g] = ps

        def stage3(g):
            r0 = g * RG
            ls = [p + pr for (p, pr) in st2.pop(g)]
            if r0 < HALO:
                rows = row0 + r0 + lax.broadcasted_iota(jnp.int32, (RG, 128), 0)
                ls = [ls[0]] + [jnp.where(rows >= DIL * w, ls[w], NEG) for w in range(1, WIN)]
            m01 = jnp.maximum(ls[0], ls[1]); m23 = jnp.maximum(ls[2], ls[3])
            m45 = jnp.maximum(ls[4], ls[5]); m67 = jnp.maximum(ls[6], ls[7])
            m = jnp.maximum(jnp.maximum(m01, m23), jnp.maximum(m45, m67))
            es = [jnp.exp2(l - m) for l in ls]
            den = ((es[0] + es[1]) + (es[2] + es[3])) + ((es[4] + es[5]) + (es[6] + es[7]))
            inv = 1.0 / den
            o = []
            for j in range(NJ):
                acc = es[0] * v_r[j, pl.ds(HALO + r0, RG), :]
                for w in range(1, WIN):
                    acc = acc + es[w] * v_r[j, pl.ds(HALO + r0 - DIL * w, RG), :]
                o.append(acc * inv)
            outs[g] = o
            if g % 2 == 1:
                o0 = outs.pop(g - 1)
                o1 = outs.pop(g)
                for j in range(NJ):
                    o_r[(g - 1) * RG:(g + 1) * RG, j * 128:(j + 1) * 128] = (
                        jnp.concatenate([o0[j], o1[j]], axis=0).astype(bf16))

        for t in range(ng + 2):
            if t < ng:
                stage1(t)
            if 0 <= t - 1 < ng:
                stage2(t - 1)
            if 0 <= t - 2 < ng:
                stage3(t - 2)

    def post(row0, o_r):
        a = jnp.dot(o_r[...], wo_p[...], preferred_element_type=f32)
        ga = mod_v[0:1, 2 * D:3 * D]
        sb = mod_v[0:1, 3 * D:4 * D]
        cb = mod_v[0:1, 4 * D:5 * D]
        gb = mod_v[0:1, 5 * D:6 * D]
        x1b = (x_v[pl.ds(row0, TM), :].astype(f32) + ga * a).astype(bf16)
        x1_v[pl.ds(row0, TM), :] = x1b
        x1 = x1b.astype(f32)
        h2b = (ln_rows(x1) * (1.0 + cb) + sb).astype(bf16)
        h2_v[pl.ds(row0, TM), :] = h2b
        h2 = h2b.astype(f32)
        out_v[pl.ds(row0, TM), :] = (x1 + gb * h2).astype(bf16)
        wr = wr_v[...].astype(f32).reshape(1, D)
        r = jnp.sum(h2 * wr, axis=-1, keepdims=True).astype(bf16).astype(f32)
        bv = best_v[...]
        bi = besti_v[...]
        sub = lax.broadcasted_iota(jnp.int32, (8, 128), 0)
        for g in range(TM // 8):
            rg = jnp.broadcast_to(r[g * 8:(g + 1) * 8], (8, 128))
            upd = rg > bv
            bv = jnp.where(upd, rg, bv)
            bi = jnp.where(upd, sub + (row0 + g * 8), bi)
        best_v[...] = bv
        besti_v[...] = bi

    def out_cp(t):
        r = t * TM
        if not isinstance(t, int):
            r = pl.multiple_of(r, TM)
        return pltpu.make_async_copy(out_v.at[pl.ds(r, TM)], out_hbm.at[pl.ds(r, TM)], osems.at[t])

    best_v[...] = jnp.full((8, 128), -jnp.inf, f32)
    besti_v[...] = jnp.zeros((8, 128), jnp.int32)
    for j in range(NJ):
        ka[j, 0:HALO, :] = jnp.zeros((HALO, 128), f32)
        va[j, 0:HALO, :] = jnp.zeros((HALO, 128), f32)
    c_cp.wait()
    wm0_cp.wait()
    mod_part(0, 2 * D)
    x0_cp.wait()
    ln1(0)
    wqkv_cp.wait()
    permute_wqkv()
    qkv(qa, ka, va)
    xr_cp.wait()
    wo_cp.wait()
    wm1_cp.wait()
    wr_cp.wait()
    permute_wo()
    mod_part(2 * D, 6 * D)
    ln1(TM)
    halo(ka, va, kb, vb)
    qkv(qb, kb, vb)
    attention(0, qa, ka, va, oa)

    def step(t, cur, nxt):
        (q_c, k_c, v_c, o_c), (q_n, k_n, v_n, o_n) = cur, nxt
        r_prev = pl.multiple_of((t - 1) * TM, TM)
        r_cur = pl.multiple_of(t * TM, TM)
        r_nxt = pl.multiple_of((t + 1) * TM, TM)
        ln1(r_nxt)
        post(r_prev, o_n)
        halo(k_c, v_c, k_n, v_n)
        qkv(q_n, k_n, v_n)
        attention(r_cur, q_c, k_c, v_c, o_c)
        out_cp(t - 1).start()

    A = (qa, ka, va, oa)
    B = (qb, kb, vb, ob)

    def body(u, carry):
        step(2 * u + 1, B, A)
        step(2 * u + 2, A, B)
        return carry

    lax.fori_loop(0, (NT - 2) // 2, body, 0)
    post((NT - 2) * TM, oa)
    attention((NT - 1) * TM, qb, kb, vb, ob)
    out_cp(NT - 2).start()
    post((NT - 1) * TM, ob)
    out_cp(NT - 1).start()

    bv = best_v[...]
    bi = besti_v[...]
    mx = jnp.max(bv, axis=0, keepdims=True)
    cand = jnp.where(bv == mx, bi, S)
    idxv = jnp.min(cand, axis=0, keepdims=True)
    idxv = jnp.minimum(idxv, S - 1)
    idx = idxv[0, 0]
    base = pl.multiple_of((idx // 16) * 16, 16)
    wg_cp.wait()
    wu_cp.wait()
    wd_cp.wait()
    hb = h2_v[pl.ds(base, 16), :]
    g = lax.dot_general(hb, wg_v[...], (((1,), (1,)), ((), ())), preferred_element_type=f32)
    u = lax.dot_general(hb, wu_v[...], (((1,), (1,)), ((), ())), preferred_element_type=f32)
    act = (g * jax.nn.sigmoid(g) * u).astype(bf16)
    y = jnp.dot(act, wd_v[...], preferred_element_type=f32)
    y = y * jax.nn.sigmoid(mx[:, 0:1])
    rows = base + lax.broadcasted_iota(jnp.int32, (16, D), 0)
    upd = jnp.where(rows == idx, y, 0.0)
    gb = mod_v[0:1, 5 * D:6 * D]
    newblk = x1_v[pl.ds(base, 16), :].astype(f32) + gb * (hb.astype(f32) + upd)
    for t in range(NT):
        out_cp(t).wait()
    out_v[pl.ds(base, 16), :] = newblk.astype(bf16)
    fix = pltpu.make_async_copy(out_v.at[pl.ds(base, 16)], out_hbm.at[pl.ds(base, 16)], sems.at[11])
    fix.start()
    fix.wait()


@jax.jit
def pallas_adaLN_cond__sliding_local_dilated__moe_arch_mod__prompt_kernel(
    A_x, A_wqkv, A_wo, B_x, B_w_r, B_w_gate, B_w_up, B_w_down, c, w_mod,
):
    x = A_x.reshape(S, D)
    wr = B_w_r
    V = pltpu.VMEM
    scratch = [
        V((S, D), bf16),
        V((D, 3 * D), bf16),
        V((D, 3 * D), bf16),
        V((D, D), bf16),
        V((NJ, D, 128), f32),
        V((D, D), bf16),
        V((F, D), bf16),
        V((F, D), bf16),
        V((F, D), bf16),
        V((D, 6 * D), bf16),
        V((1, D), bf16),
        V((D,), bf16),
        V((8, 6 * D), f32),
        V((TM, D), bf16),
        V((NJ, TM, 128), f32), V((NJ, TM, 128), f32),
        V((NJ, TM + HALO, 128), f32), V((NJ, TM + HALO, 128), f32),
        V((NJ, TM + HALO, 128), f32), V((NJ, TM + HALO, 128), f32),
        V((TM, D), bf16), V((TM, D), bf16),
        V((S, D), bf16),
        V((S, D), bf16),
        V((S, D), bf16),
        V((8, 128), f32),
        V((8, 128), jnp.int32),
        pltpu.SemaphoreType.DMA((12,)),
        pltpu.SemaphoreType.DMA((NT,)),
    ]
    out = pl.pallas_call(
        _kernel,
        out_shape=jax.ShapeDtypeStruct((S, D), bf16),
        in_specs=[pl.BlockSpec(memory_space=pltpu.HBM)] * 9,
        out_specs=pl.BlockSpec(memory_space=pltpu.HBM),
        scratch_shapes=scratch,
        compiler_params=pltpu.CompilerParams(vmem_limit_bytes=100 * 2**20),
    )(x, A_wqkv, A_wo, wr, B_w_gate.T, B_w_up.T, B_w_down, c, w_mod)
    return out.reshape(1, S, D)
```

```python
import math

import jax
import jax.numpy as jnp
from jax import lax
import jax.experimental.pallas as pl
import jax.experimental.pallas.tpu as pltpu


S = 2048
D = 640
H = 32
DH = 20
WIN = 8
F = 1728
NJ = D // 128
TM = 256
NT = S // TM
NG = TM // 8
HV = 14
MS = 64
NM = TM // MS
GM = MS // 8
KVR = (HV + NG + 1) * 8
EPS = 1e-5
LOG2E = math.log2(math.e)
QSCALE = (DH ** -0.5) * LOG2E
NEG = -1000000000.0 * LOG2E
f32 = jnp.float32
bf16 = jnp.bfloat16
u32 = jnp.uint32
i32 = jnp.int32

WA = 12
WL = 8
WP = 8
CH = 2
ATHI = 70
LNHI = 76
POLO = 24
POHI = 74


def _spread(n, lo, hi):
    return [int(lo + (i * (hi - lo)) / n) for i in range(n)]


def _kernel(x_hbm, wqkv_hbm, wo_hbm, wr_hbm, wg_hbm, wu_hbm, wd_hbm, c_hbm, wmod_hbm,
            out_hbm,
            x_v, wqkv_raw, wo_raw, wo_f, wg_v, wu_v, wd_v, wmod_v, c_v, wr_v,
            mod_v, ha, hb, qa, qb, ka, kb, va, vb, oa, ob, x1a, x1b, h2_v, out_v, best_v, besti_v,
            zsrc, zero_v, zs, sems, osems, *wp):
    wq_p = wp[:15]
    wo_p = wp[15:20]

    def cp(src, dst, i):
        return pltpu.make_async_copy(src, dst, sems.at[i])

    def xcp(t0, nt, i):
        return cp(x_hbm.at[pl.ds(t0 * TM, nt * TM)], x_v.at[pl.ds(t0 * TM, nt * TM)], i)

    def wmcp(k0, nk, i):
        return cp(wmod_hbm.at[:, pl.ds(k0 * D, nk * D)], wmod_v.at[:, pl.ds(k0 * D, nk * D)], i)

    def wqcp(t, i):
        return cp(wqkv_hbm.at[:, pl.ds(t * D, D)], wqkv_raw.at[:, pl.ds(t * D, D)], i)

    c_cp = cp(c_hbm, c_v, 0)
    x0_cp = xcp(0, 1, 1)
    wm0_cp = wmcp(0, 2, 2)
    wq_cps = [wqcp(t, 3 + t) for t in range(3)]
    x1_cp = xcp(1, 1, 6)
    x2_cp = xcp(2, 1, 7)
    wo_cp = cp(wo_hbm, wo_raw, 8)
    wm1_cp = wmcp(2, 1, 9)
    wm2_cp = wmcp(3, 3, 10)
    wr_cp = cp(wr_hbm, wr_v, 11)
    x3_cp = xcp(3, 1, 12)
    xr_cp = xcp(4, 4, 13)
    wg_cp = cp(wg_hbm, wg_v, 14)
    wu_cp = cp(wu_hbm, wu_v, 15)
    wd_cp = cp(wd_hbm, wd_v, 16)
    z_cp = cp(zsrc, zero_v, 17)
    zsrc[...] = jnp.zeros((8, 128), u32)
    for d in [c_cp, z_cp, x0_cp, wm0_cp] + wq_cps + [x1_cp, x2_cp, wo_cp, wm1_cp, wm2_cp, wr_cp, x3_cp, xr_cp,
                                               wg_cp, wu_cp, wd_cp]:
        d.start()

    def tob(u):
        return pltpu.bitcast(u, bf16)

    def tou(b):
        return pltpu.bitcast(b, u32)

    def pack2(a, b):
        return pltpu.bitcast(pltpu.pack_elementwise([a, b], packed_dtype=bf16), u32)

    def zand(v):
        return pltpu.bitcast(v, u32) & zero_v[...]

    def orall(vs):
        r = vs[0]
        for v in vs[1:]:
            r = r | v
        return r

    def mrow(k, j):
        return mod_v[:, k * D + j * 128:k * D + (j + 1) * 128]

    def tree(vs):
        return ((vs[0] + vs[1]) + (vs[2] + vs[3])) + vs[4]

    def lsum(v):
        return jnp.sum(v, axis=-1, keepdims=True)

    def stats(s, s2):
        m = s * (1.0 / D)
        v = jnp.maximum(s2 * (1.0 / D) - m * m, 0.0)
        return m, lax.rsqrt(v + EPS)

    def zo(i):
        return pl.multiple_of(zs[i], 8)

    def gated(w, toks):
        if toks:
            t = orall(toks) & zero_v[...]
            w = jnp.concatenate([w[0:8] | t, w[8:]], axis=0)
        return tob(w)

    def lhs(ref, m):
        return tob(jnp.concatenate([ref[j, m * MS // 2:(m + 1) * MS // 2] for j in range(NJ)], axis=1))

    def job_qkv(buf, n, m):
        h_r, q_r, k_r, v_r = buf[0], buf[1], buf[2], buf[3]

        def run(toks):
            res = jnp.dot(lhs(h_r, m), gated(wq_p[n][pl.ds(zo(m), D // 2), :], toks),
                          preferred_element_type=f32)
            if n < NJ:
                q_r[n, m * MS:(m + 1) * MS, :] = res
            elif n < 2 * NJ:
                k_r[n - NJ, HV * 8 + m * MS:HV * 8 + (m + 1) * MS, :] = res
            else:
                v_r[n - 2 * NJ, HV * 8 + m * MS:HV * 8 + (m + 1) * MS, :] = res
            return res[0:8]
        return run

    def job_wo(o_r, x1_r, row0, c, m):
        def run(toks):
            a = jnp.dot(lhs(o_r, m), gated(wo_p[c][pl.ds(zo(m), D // 2), :], toks),
                        preferred_element_type=f32)
            ga = mrow(2, c)
            for ci in range(GM):
                cc = m * GM + ci
                g = 4 * (cc % 8) + cc // 8
                xr = x_v[pl.ds(row0 + g * 8, 8), c * 128:(c + 1) * 128].astype(f32)
                x1_r[c, g * 8:(g + 1) * 8, :] = xr + ga * a[ci * 8:(ci + 1) * 8]
            return a[0:8]
        return run

    def silu_c():
        c = c_v[...].astype(f32)
        sc = (c * jax.nn.sigmoid(c)).astype(bf16)
        return jnp.broadcast_to(sc, (16, D))

    def job_mod(k, j, w=128):
        def run(toks):
            lo = k * D + j * 128
            m = jnp.dot(silu_c(), wmod_v[:, lo:lo + w], preferred_element_type=f32)
            m = m[:8].astype(bf16).astype(f32)
            if k in (1, 4):
                m = m + 1.0
            mod_v[:, lo:lo + w] = m
            return None
        return run

    def job_call(fn):
        def run(toks):
            fn()
            return None
        return run

    def st_attention(buf, slots, fin, first=False, order=None):
        q_c, k_c, v_c, o_c = buf[1], buf[2], buf[3], buf[4]
        st1, st2, outs, chain = {}, {}, {}, []
        order = order or [(i + HV) % NG for i in range(NG)]

        def ld(ref, j, i):
            return ref[j, (HV + i) * 8:(HV + i + 1) * 8, :]

        def a1(g, tok):
            if CH and len(chain) >= CH:
                ct = zand(chain[-CH])
                tok = ct if tok is None else tok | ct
            sc = QSCALE if tok is None else pltpu.bitcast(
                pltpu.bitcast(jnp.full((8, 128), QSCALE, f32), u32) | tok, f32)
            q = [q_c[j, g * 8:(g + 1) * 8, :] * sc for j in range(NJ)]
            ps = []
            for w in range(WIN):
                p = q[0] * ld(k_c, 0, g - 2 * w)
                for j in range(1, NJ):
                    p = p + q[j] * ld(k_c, j, g - 2 * w)
                ps.append((p, pltpu.roll(p, 64, 1)))
            st1[g] = ps

        def a2(g):
            ps = []
            for (p, pr) in st1.pop(g):
                p = p + pr
                ps.append((p, pltpu.roll(p, 32, 1)))
            st2[g] = ps

        def a3(g, dl):
            ls = [p + pr for (p, pr) in st2.pop(g)]
            if first:
                sub = lax.broadcasted_iota(i32, (8, 128), 0)
                ls = [jnp.where(sub > 0, ls[w], NEG) if g - 2 * w < 0 else ls[w] for w in range(WIN)]
            m = jnp.maximum(jnp.maximum(jnp.maximum(ls[0], ls[1]), jnp.maximum(ls[2], ls[3])),
                            jnp.maximum(jnp.maximum(ls[4], ls[5]), jnp.maximum(ls[6], ls[7])))
            es = [jnp.exp2(l - m) for l in ls]
            den = ((es[0] + es[1]) + (es[2] + es[3])) + ((es[4] + es[5]) + (es[6] + es[7]))
            inv = pl.reciprocal(den, approx=True)
            o = []
            for j in range(NJ):
                acc = es[0] * ld(v_c, j, g)
                for w in range(1, WIN):
                    acc = acc + es[w] * ld(v_c, j, g - 2 * w)
                o.append(acc * inv)
            outs[g] = o
            chain.append(o[NJ - 1])
            if g % 2 == 1:
                o0 = outs.pop(g - 1)
                o1 = outs.pop(g)
                pk = [pack2(o0[j], o1[j]) for j in range(NJ)]
                for j in range(NJ):
                    o_c[j, pl.ds(32 * (g // 8) + (g // 2) % 4, 8, stride=4), :] = pk[j]
                fin(dl, orall(pk))

        def emit(i, tk):
            if i < NG:
                a1(order[i], tk())
            if 0 <= i - 1 < NG:
                a2(order[i - 1])
            if 0 <= i - 2 < NG:
                a3(order[i - 2], slots[i - 2] + WA)
        return slots + [slots[-1] + 1, slots[-1] + 2], emit

    def st_halo(cur, prv, slots):
        def emit(i, tk):
            dst = cur[2] if i < NJ else cur[3]
            j = i % NJ
            sub = lax.broadcasted_iota(i32, (8, 128), 0)
            tok = tk()
            if tok is not None:
                sub = sub | pltpu.bitcast(tok, i32)
            for m in range(1, HV + 1):
                a0 = (HV + NG - m) * 8
                if prv is None:
                    top = 0.0
                else:
                    src = prv[2] if i < NJ else prv[3]
                    top = src[j, a0 + 7:a0 + 15, :]
                dst[j, (HV - m) * 8:(HV - m + 1) * 8, :] = jnp.where(sub < 1, top, dst[j, a0 - 1:a0 + 7, :])
        return slots, emit

    def st_ln1(h_r, row0, slots, fin):
        l1, hs = {}, {}

        def ldx(g, z):
            r = 64 * (g // 8) + 8 * ((g // 2) % 4) + 32 * (g % 2)
            return [x_v[pl.ds(row0 + z + r, 8), j * 128:(j + 1) * 128].astype(f32) for j in range(NJ)]

        def n1(g, tok):
            xf = ldx(g, 0)
            if tok is not None:
                xf[0] = xf[0] + pltpu.bitcast(tok, f32)
            l1[g] = (lsum(tree(xf)), lsum(tree([x * x for x in xf])))

        def n3(g, dl):
            m, rs = stats(*l1.pop(g))
            xf = ldx(g, zo(0))
            hs[g] = [(xf[j] - m) * rs * mrow(1, j) + mrow(0, j) for j in range(NJ)]
            if g % 2 == 1:
                b = g // 2
                h0 = hs.pop(g - 1)
                h1 = hs.pop(g)
                pk = [pack2(h0[j], h1[j]) for j in range(NJ)]
                for j in range(NJ):
                    h_r[j, pl.ds(32 * (b % 4) + b // 4, 8, stride=4), :] = pk[j]
                fin(dl, orall(pk))

        def emit(i, tk):
            if i < NG:
                n1(i, tk())
            if 0 <= i - 1 < NG:
                n3(i - 1, slots[i - 1] + WL)
        return slots + [slots[-1] + 1], emit

    def st_post(x1_r, row0, slots, fin, order=None):
        p1s, p3s, bst = {}, {}, {}
        natural = order is None
        order = order or list(range(NG))

        def ldx1(g, z):
            return [x1_r[j, pl.ds(g * 8 + zo(z), 8), :] for j in range(NJ)]

        def p1(g, tok):
            xf = ldx1(g, 0)
            if tok is not None:
                xf[0] = xf[0] + pltpu.bitcast(tok, f32)
            p1s[g] = (lsum(tree(xf)), lsum(tree([x * x for x in xf])))

        def p3(g, dl):
            x1 = ldx1(g, 1)
            m, rs = stats(*p1s.pop(g))
            h2 = [(x1[j] - m) * rs * mrow(4, j) + mrow(3, j) for j in range(NJ)]
            ov = [x1[j] + mrow(5, j) * h2[j] for j in range(NJ)]
            p3s[g] = lsum(tree([h2[j] * mrow(6, j) for j in range(NJ)]))
            h2_v[pl.ds(row0 + g * 8, 8), :] = jnp.concatenate(h2, axis=1)
            out_v[pl.ds(row0 + g * 8, 8), :] = jnp.concatenate(ov, axis=1).astype(bf16)
            fin(dl, orall([pltpu.bitcast(o, u32) for o in ov]))

        def p4(g, n, dl):
            r = p3s.pop(g).astype(bf16).astype(f32)
            if n == 0:
                bst['v'] = best_v[...]
                bst['i'] = besti_v[...]
            rg = jnp.broadcast_to(r, (8, 128))
            upd = rg > bst['v']
            if not natural:
                upd = upd | ((rg == bst['v']) & (bst['i'] > row0 + g * 8))
            bst['v'] = jnp.where(upd, rg, bst['v'])
            bst['i'] = jnp.where(upd, row0 + g * 8, bst['i'])
            if n == NG - 1:
                best_v[...] = bst['v']
                besti_v[...] = bst['i']
            if n % 2 == 1:
                fin(dl, pltpu.bitcast(bst['i'], u32))

        def emit(i, tk):
            if i < NG:
                p1(order[i], tk())
            if 0 <= i - 1 < NG:
                p3(order[i - 1], slots[i - 1] + WP)
            if 0 <= i - 2 < NG:
                p4(order[i - 2], i - 2, slots[i - 2] + WP + 2)
        return slots + [slots[-1] + 1, slots[-1] + 2], emit

    def perm_q(n):
        t, j = n // NJ, n % NJ
        lane = lax.broadcasted_iota(i32, (8, 128), 1)
        quad = lane // 4
        idx = 4 * ((5 * (lane % 32) + j) % 32) + lane // 32
        src_blk = ((j + 5 * 32 - quad) * 3) % 5
        masks = [src_blk == i for i in range(1, NJ)]
        for r in range(D // 16):
            srcs = [tou(wqkv_raw[r * 16:(r + 1) * 16, t * D + i * 128:t * D + (i + 1) * 128])
                    for i in range(NJ)]
            m = srcs[0]
            for i in range(1, NJ):
                m = jnp.where(masks[i - 1], srcs[i], m)
            wq_p[n][r * 8:(r + 1) * 8, :] = jnp.take_along_axis(m, idx, axis=1)

    def perm_o(n):
        wo_f[n] = wo_raw[:, n * 128:(n + 1) * 128].astype(f32)
        for j in range(NJ):
            for dd in range(4):
                for hh in range(2):
                    r0 = hh * 16 * DH + 4 * j + dd
                    ev = wo_f[n, pl.ds(r0, 8, stride=2 * DH), :]
                    od = wo_f[n, pl.ds(r0 + DH, 8, stride=2 * DH), :]
                    p0 = j * 64 + dd * 16 + hh * 8
                    wo_p[n][p0:p0 + 8, :] = pack2(ev, od)

    class Phase:
        def __init__(self, carry=None):
            self.done = {}
            self.tok = None
            if carry is not None:
                self.done = dict(carry.left)
                self.tok = carry.tok
            self.cur = 0

        def fin(self, slot, v):
            self.done.setdefault(max(slot, self.cur), []).append(v)

        def run(self, jobs, streams):
            pos = [0] * len(streams)
            pend = []
            for c in range(len(jobs) + 1):
                self.cur = c
                cache = []

                def tk():
                    if self.tok is None:
                        return None
                    if not cache:
                        cache.append(zand(self.tok))
                    return cache[0]
                for si, (slots, emit) in enumerate(streams):
                    while pos[si] < len(slots) and (slots[pos[si]] <= c or c == len(jobs)):
                        emit(pos[si], tk)
                        pos[si] += 1
                if c == len(jobs):
                    break
                pend += self.done.pop(c, [])
                r = jobs[c](pend)
                if r is not None:
                    self.tok = r
                    pend = []
            self.left = {k - len(jobs): v for k, v in self.done.items()}

    def out_cp(t, nt, i):
        r = t * TM
        if not isinstance(t, int):
            r = pl.multiple_of(r, TM)
        return pltpu.make_async_copy(out_v.at[pl.ds(r, nt * TM)], out_hbm.at[pl.ds(r, nt * TM)], osems.at[i])

    A = (ha, qa, ka, va, oa)
    B = (hb, qb, kb, vb, ob)

    def qkv_jobs(buf, ns):
        return [job_qkv(buf, n, m) for n in ns for m in range(NM)]

    best_v[...] = jnp.full((8, 128), -jnp.inf, f32)
    besti_v[...] = jnp.zeros((8, 128), i32)
    for r_ in (ka, kb, va, vb):
        for j in range(NJ):
            r_[j, KVR - 8:KVR, :] = jnp.zeros((8, 128), f32)
    z_cp.wait()
    zv = pltpu.bitcast(zero_v[...], i32)
    for i in range(4):
        zs[i] = zv[i, 0]
    c_cp.wait()
    x0_cp.wait()
    wm0_cp.wait()
    job_mod(0, 0, D)([])
    job_mod(1, 0, D)([])
    ph = Phase()
    ph.run([], [st_ln1(ha, 0, [0] * NG, ph.fin)])

    ph = Phase()
    jobs = []
    for t in range(3):
        jobs.append(job_call(wq_cps[t].wait))
        for j in range(NJ):
            jobs.append(job_call(lambda n=t * NJ + j: perm_q(n)))
            if t == 2 and j == 1:
                jobs.append(job_call(x1_cp.wait))
                ln_lo = len(jobs)
            jobs += qkv_jobs(A, [t * NJ + j])
    ph.run(jobs, [st_ln1(hb, TM, _spread(NG, ln_lo, len(jobs) - 6), ph.fin)])

    x2_cp.wait()
    ph = Phase()
    jobs = qkv_jobs(B, range(8))
    jobs += [job_call(wo_cp.wait), job_call(wm1_cp.wait)]
    for n in range(8, 13):
        jobs += [job_call(lambda n=n: perm_o(n - 8)), job_mod(2, n - 8)] + qkv_jobs(B, [n])
    jobs += qkv_jobs(B, [13, 14])
    nj = len(jobs)
    ph.run(jobs, [st_halo(A, None, _spread(10, 1, 12)),
                  st_attention(A, _spread(NG, 0, nj - 10), ph.fin, first=True),
                  st_ln1(ha, 2 * TM, _spread(NG, 0, nj - 4), ph.fin)])

    ph = Phase(ph)
    jobs = [job_wo(oa, x1a, 0, c, m) for c in range(NJ) for m in range(NM)]
    jobs += qkv_jobs(A, range(5))

    def wr_setup():
        wm2_cp.wait()
        wr_cp.wait()
        x3_cp.wait()
        mod_v[:, 6 * D:7 * D] = jnp.broadcast_to(wr_v[...].astype(f32).reshape(1, D), (8, D))
    jobs += [job_call(wr_setup)]
    w1 = len(jobs)
    for i in range(8):
        jobs += [job_mod(3 + k // NJ, k % NJ) for k in range(2 * i, min(2 * i + 2, 15))]
        jobs += [job_qkv(A, 5 + i // NM, i % NM)]
    w2 = len(jobs)
    jobs += qkv_jobs(A, range(7, 15))
    nj = len(jobs)
    ph.run(jobs, [st_halo(B, A, _spread(10, 2, 18)),
                  st_attention(B, _spread(22, 0, w1) + _spread(10, w2 - 4, nj - 10), ph.fin),
                  st_ln1(hb, 3 * TM, _spread(NG, w1, nj - 4), ph.fin),
                  st_post(x1a, 0, _spread(NG, w2, nj - 5), ph.fin)])
    out_cp(0, 1, 0).start()
    xr_cp.wait()

    def step(t, cur, nxt, carry):
        r_prev = pl.multiple_of((t - 1) * TM, TM)
        r_nn = pl.multiple_of((t + 2) * TM, TM)
        ph = Phase(carry)
        jobs = [job_wo(nxt[4], x1a, r_prev, c, m) for c in range(NJ) for m in range(NM)]
        jobs += qkv_jobs(nxt, range(15))
        ph.run(jobs, [st_halo(cur, nxt, _spread(10, 2, 18)),
                      st_attention(cur, _spread(NG, 0, ATHI), ph.fin),
                      st_ln1(cur[0], r_nn, _spread(NG, 0, LNHI), ph.fin),
                      st_post(x1a, r_prev, _spread(NG, POLO, POHI), ph.fin)])
        return ph

    def body(u, carry):
        ph = step(2 * u + 2, A, B, None)
        step(2 * u + 3, B, A, ph)
        out_cp(2 * u + 1, 2, u + 1).start()
        return carry

    lax.fori_loop(0, 2, body, 0)

    ph = Phase()
    mord = [4 * (cc % 8) + cc // 8 for cc in range(NG)]
    jobs = [job_wo(ob, x1a, 5 * TM, c, m) for c in range(NJ) for m in range(NM)]
    jobs += qkv_jobs(B, range(5, 15))
    jobs += [job_qkv(B, n, m) for m in range(NM) for n in range(NJ)]
    jobs += [job_wo(oa, x1b, 6 * TM, c, m) for m in range(NM) for c in range(NJ)]
    jobs += [job_wo(ob, x1a, 7 * TM, c, m) for m in range(NM) for c in range(NJ)]
    T1 = 58; T2 = 67; T3 = 104
    ph.run(jobs, [st_halo(A, B, _spread(10, 2, 18)),
                  st_attention(A, _spread(NG, 0, T1), ph.fin),
                  st_post(x1a, 5 * TM, _spread(NG, 24, 66), ph.fin),
                  st_halo(B, A, _spread(5, 44, 54) + _spread(5, 62, 66)),
                  st_attention(B, _spread(NG, T2, T3), ph.fin, order=list(range(NG))),
                  st_post(x1b, 6 * TM, _spread(NG, 87, 112), ph.fin, order=mord),
                  st_post(x1a, 7 * TM, [max(113, 107 + 5 * (i // 8)) for i in range(NG)], ph.fin, order=mord)])
    out_cp(5, 3, 3).start()

    bv = best_v[...]
    bi = besti_v[...] + lax.broadcasted_iota(i32, (8, 128), 0)
    mx = jnp.max(bv, axis=0, keepdims=True)
    cand = jnp.where(bv == mx, bi, S)
    idxv = jnp.min(cand, axis=0, keepdims=True)
    idxv = jnp.minimum(idxv, S - 1)
    idx = idxv[0, 0]
    base = pl.multiple_of((idx // 16) * 16, 16)
    wg_cp.wait()
    wu_cp.wait()
    wd_cp.wait()
    hb16 = h2_v[pl.ds(base, 16), :].astype(bf16)
    g = lax.dot_general(hb16, wg_v[...], (((1,), (1,)), ((), ())), preferred_element_type=f32)
    u = lax.dot_general(hb16, wu_v[...], (((1,), (1,)), ((), ())), preferred_element_type=f32)
    act = (g * jax.nn.sigmoid(g) * u).astype(bf16)
    y = jnp.dot(act, wd_v[...], preferred_element_type=f32)
    y = y * jax.nn.sigmoid(mx[:, 0:1])
    rows = base + lax.broadcasted_iota(i32, (16, D), 0)
    gb = mod_v[0:1, 5 * D:6 * D]
    old = out_v[pl.ds(base, 16), :].astype(f32)
    newblk = jnp.where(rows == idx, old + gb * y, old)
    out_cp(0, 1, 0).wait()
    out_cp(1, 2, 1).wait()
    out_cp(3, 2, 2).wait()
    out_cp(5, 3, 3).wait()
    out_v[pl.ds(base, 16), :] = newblk.astype(bf16)
    fix = pltpu.make_async_copy(out_v.at[pl.ds(base, 16)], out_hbm.at[pl.ds(base, 16)], sems.at[18])
    fix.start()
    fix.wait()


@jax.jit
def pallas_adaLN_cond__sliding_local_dilated__moe_arch_mod__prompt_kernel(
    A_x, A_wqkv, A_wo, B_x, B_w_r, B_w_gate, B_w_up, B_w_down, c, w_mod,
):
    x = A_x.reshape(S, D)
    V = pltpu.VMEM
    scratch = [
        V((S, D), bf16),
        V((D, 3 * D), bf16),
        V((D, D), bf16),
        V((NJ, D, 128), f32),
        V((F, D), bf16),
        V((F, D), bf16),
        V((F, D), bf16),
        V((D, 6 * D), bf16),
        V((1, D), bf16),
        V((D,), bf16),
        V((8, 7 * D), f32),
        V((NJ, TM // 2, 128), u32), V((NJ, TM // 2, 128), u32),
        V((NJ, TM, 128), f32), V((NJ, TM, 128), f32),
        V((NJ, KVR, 128), f32), V((NJ, KVR, 128), f32),
        V((NJ, KVR, 128), f32), V((NJ, KVR, 128), f32),
        V((NJ, TM // 2, 128), u32), V((NJ, TM // 2, 128), u32),
        V((NJ, TM, 128), f32), V((NJ, TM, 128), f32),
        V((S, D), f32),
        V((S, D), bf16),
        V((8, 128), f32),
        V((8, 128), i32),
        V((8, 128), u32),
        V((8, 128), u32),
        pltpu.SMEM((4,), i32),
        pltpu.SemaphoreType.DMA((19,)),
        pltpu.SemaphoreType.DMA((4,)),
    ] + [V((D // 2, 128), u32)] * 20
    out = pl.pallas_call(
        _kernel,
        out_shape=jax.ShapeDtypeStruct((S, D), bf16),
        in_specs=[pl.BlockSpec(memory_space=pltpu.HBM)] * 9,
        out_specs=pl.BlockSpec(memory_space=pltpu.HBM),
        scratch_shapes=scratch,
        compiler_params=pltpu.CompilerParams(vmem_limit_bytes=100 * 2**20),
    )(x, A_wqkv, A_wo, B_w_r, B_w_gate.T, B_w_up.T, B_w_down, c, w_mod)
    return out.reshape(1, S, D)
```

```python
import math

import jax
import jax.numpy as jnp
from jax import lax
import jax.experimental.pallas as pl
import jax.experimental.pallas.tpu as pltpu


S = 2048
D = 640
H = 32
DH = 20
WIN = 8
F = 1728
NJ = D // 128
TM = 256
NT = S // TM
NG = TM // 8
HV = 14
MS = 64
NM = TM // MS
GM = MS // 8
KVR = (HV + NG + 1) * 8
EPS = 1e-5
LOG2E = math.log2(math.e)
QSCALE = (DH ** -0.5) * LOG2E
NEG = -1000000000.0 * LOG2E
f32 = jnp.float32
bf16 = jnp.bfloat16
u32 = jnp.uint32
i32 = jnp.int32
NSEM = 12

WA = 12
WL = 8
WP = 8
CH = 2
ATHI = 8
LNHI = 4
POLO = 7
PL7 = 6
PT = 0
SNAP = 2


def _spread(n, lo, hi):
    return [int(lo + (i * (hi - lo)) / n) for i in range(n)]


def _kernel(x_hbm, wqkv_hbm, wo_hbm, wr_hbm, wg_hbm, wu_hbm, wd_hbm, c_hbm, wmod_hbm,
            out_hbm, *wp):
    (x_3, bias_v, wqkv_raw, wo_raw, wo_f, wg_v, wu_v, wd_v, wmod_v,
     mod_v, ha, hb, qa, qb, ka, kb, va, vb, o_all, oc, h2_v, out_v, best_v, besti_v,
     zsrc, zero_v, sc_v, sap_v, fix_v, c_v, wr_v, zs, sems) = wp[28:]
    x_v = x_3.at[0]
    wq_p = wp[:15]
    wo_p = wp[15:20]
    x1s = wp[20:28]

    def cp(src, dst, i):
        return [pltpu.make_async_copy(src, dst, sems.at[i])]

    def xcp(t0, nt, i):
        return cp(x_hbm.at[pl.ds(t0 * TM, nt * TM)], x_v.at[pl.ds(t0 * TM, nt * TM)], i)

    def colcp(src, dst, k0, nk, i):
        return cp(src.at[:, pl.ds(k0 * D, nk * D)], dst.at[:, pl.ds(k0 * D, nk * D)], i)

    def wait(g):
        for d in g:
            d.wait()

    g_z = cp(zsrc, zero_v, 0)
    g_x0 = xcp(0, 2, 1) + cp(c_hbm, c_v, 1)
    g_wq = colcp(wqkv_hbm, wqkv_raw, 0, 1, 2)
    g_ca = colcp(wmod_hbm, wmod_v, 1, 1, 3)
    g_wk = colcp(wqkv_hbm, wqkv_raw, 1, 1, 4)
    g_wv = colcp(wqkv_hbm, wqkv_raw, 2, 1, 5) + colcp(wmod_hbm, wmod_v, 0, 1, 5)
    g_xr = xcp(2, 6, 6)
    g_rest = (colcp(wmod_hbm, wmod_v, 2, 4, 7) + cp(wo_hbm, wo_raw, 11) + cp(wr_hbm, wr_v, 11)
              + cp(wg_hbm, wg_v, 8) + cp(wu_hbm, wu_v, 9) + cp(wd_hbm, wd_v, 11))
    zsrc[...] = jnp.zeros((8, 128), u32)
    for d in g_x0 + g_wq + g_ca + g_z + g_wk + g_wv + g_xr + g_rest:
        d.start()

    BUF = [(ha, qa, ka, va), (hb, qb, kb, vb)]

    def tob(u):
        return pltpu.bitcast(u, bf16)

    def tou(b):
        return pltpu.bitcast(b, u32)

    def pack2(a, b):
        return pltpu.bitcast(pltpu.pack_elementwise([a, b], packed_dtype=bf16), u32)

    def zand(v):
        return pltpu.bitcast(v, u32) & zero_v[...]

    def orall(vs):
        r = vs[0]
        for v in vs[1:]:
            r = r | v
        return r

    def mrow(k, j):
        return mod_v[:, k * D + j * 128:k * D + (j + 1) * 128]

    def tree(vs):
        return ((vs[0] + vs[1]) + (vs[2] + vs[3])) + vs[4]

    def lsum(v):
        return jnp.sum(v, axis=-1, keepdims=True)

    def stats(s, s2):
        m = s * (1.0 / D)
        v = jnp.maximum(s2 * (1.0 / D) - m * m, 0.0)
        return m, jnp.exp2(jnp.log(v + EPS) * (-0.5 * LOG2E))

    def zo(i):
        return pl.multiple_of(zs[i], 8)

    def oref(t):
        return oc if t == NT - 1 else o_all.at[t]

    def gated(w, toks):
        if toks:
            t = orall(toks) & zero_v[...]
            w = jnp.concatenate([w[0:8] | t, w[8:]], axis=0)
        return tob(w)

    def lhs(ref, m, extra=None):
        a = jnp.concatenate([ref[j, m * MS // 2:(m + 1) * MS // 2] for j in range(NJ)], axis=1)
        if extra is not None:
            a = jnp.concatenate([a, extra], axis=0)
        return tob(a)

    def job_qkv(t, n, m, bias=0):
        h_r, q_r, k_r, v_r = BUF[t % 2]

        def run(toks):
            res = jnp.dot(lhs(h_r, m, sap_v[...] if bias == 1 else None),
                          gated(wq_p[n][pl.ds(zo(m), D // 2), :], toks),
                          preferred_element_type=f32)
            if bias:
                if bias == 1:
                    bb = res[MS:MS + 8]
                    bias_v[n] = bb
                else:
                    bb = bias_v[n, pl.ds(zo(m), 8), :]
                res = jnp.concatenate([res[i * 8:(i + 1) * 8] + bb for i in range(GM)], axis=0)
            if n < NJ:
                q_r[n, m * MS:(m + 1) * MS, :] = res
            elif n < 2 * NJ:
                k_r[n - NJ, HV * 8 + m * MS:HV * 8 + (m + 1) * MS, :] = res
            else:
                v_r[n - 2 * NJ, HV * 8 + m * MS:HV * 8 + (m + 1) * MS, :] = res
            return res[0:8]
        return run

    def job_bq(n):
        def run(toks):
            bias_v[n] = jnp.dot(tob(sap_v[...]), tob(wq_p[n][pl.ds(zo(0), D // 2), :]),
                                preferred_element_type=f32)[0:8]
            return None
        return run

    def job_wo(t, c, m):
        o_r, x1_r, row0 = oref(t), x1s[4 * (t % 2) + m], t * TM

        def run(toks):
            a = jnp.dot(lhs(o_r, m), gated(wo_p[c][pl.ds(zo(m), D // 2), :], toks),
                        preferred_element_type=f32)
            for ci in range(GM):
                cc = m * GM + ci
                g = 4 * (cc % 8) + cc // 8
                xr = x_v[pl.ds(row0 + g * 8, 8), c * 128:(c + 1) * 128].astype(f32)
                x1_r[c, ci * 8:(ci + 1) * 8, :] = xr + a[ci * 8:(ci + 1) * 8]
            return a[0:8]
        return run

    def job_mod(k, j):
        def run(toks):
            lo = k * D + j * 128
            m = jnp.dot(tob(sc_v[...]), wmod_v[:, lo:lo + 128], preferred_element_type=f32).astype(bf16)
            if k == 0:
                sap_v[:, j * 128:(j + 1) * 128] = tou(m)
            m = m[:8].astype(f32)
            if k in (1, 4):
                m = m + 1.0
            mod_v[:, lo:lo + 128] = m
            return None
        return run

    def job_call(fn):
        def run(toks):
            fn()
            return None
        return run

    def st_attention(t, slots, fin, order=None):
        _, q_c, k_c, v_c = BUF[t % 2]
        o_c = oref(t)
        first = t == 0
        st1, st2, outs, chain = {}, {}, {}, []
        order = order or [(i + HV) % NG for i in range(NG)]

        def ld(ref, j, i):
            return ref[j, (HV + i) * 8:(HV + i + 1) * 8, :]

        def a1(g, tok):
            if CH and len(chain) >= CH:
                ct = zand(chain[-CH])
                tok = ct if tok is None else tok | ct
            sc = QSCALE if tok is None else pltpu.bitcast(
                pltpu.bitcast(jnp.full((8, 128), QSCALE, f32), u32) | tok, f32)
            if t < 2:
                q = [(q_c[j, g * 8:(g + 1) * 8, :] + bias_v[j, pl.ds(zo(0), 8), :]) * sc for j in range(NJ)]
            else:
                q = [q_c[j, g * 8:(g + 1) * 8, :] * sc for j in range(NJ)]
            ps = []
            for w in range(WIN):
                p = q[0] * ld(k_c, 0, g - 2 * w)
                for j in range(1, NJ):
                    p = p + q[j] * ld(k_c, j, g - 2 * w)
                ps.append((p, pltpu.roll(p, 64, 1)))
            st1[g] = ps

        def a2(g):
            ps = []
            for (p, pr) in st1.pop(g):
                p = p + pr
                ps.append((p, pltpu.roll(p, 32, 1)))
            st2[g] = ps

        def a3(g, dl):
            ls = [p + pr for (p, pr) in st2.pop(g)]
            if first:
                sub = lax.broadcasted_iota(i32, (8, 128), 0)
                ls = [jnp.where(sub > 0, ls[w], NEG) if g - 2 * w < 0 else ls[w] for w in range(WIN)]
            m = jnp.maximum(jnp.maximum(jnp.maximum(ls[0], ls[1]), jnp.maximum(ls[2], ls[3])),
                            jnp.maximum(jnp.maximum(ls[4], ls[5]), jnp.maximum(ls[6], ls[7])))
            es = [jnp.exp2(l - m) for l in ls]
            den = ((es[0] + es[1]) + (es[2] + es[3])) + ((es[4] + es[5]) + (es[6] + es[7]))
            inv = pl.reciprocal(den, approx=True)
            o = []
            for j in range(NJ):
                acc = es[0] * ld(v_c, j, g)
                for w in range(1, WIN):
                    acc = acc + es[w] * ld(v_c, j, g - 2 * w)
                o.append(acc * inv)
            outs[g] = o
            chain.append(o[NJ - 1])
            if g % 2 == 1:
                o0 = outs.pop(g - 1)
                o1 = outs.pop(g)
                pk = [pack2(o0[j], o1[j]) for j in range(NJ)]
                for j in range(NJ):
                    o_c[j, pl.ds(32 * (g // 8) + (g // 2) % 4, 8, stride=4), :] = pk[j]
                fin(dl, orall(pk))

        def emit(i, tk):
            if i < NG:
                a1(order[i], tk())
            if 0 <= i - 1 < NG:
                a2(order[i - 1])
            if 0 <= i - 2 < NG:
                a3(order[i - 2], slots[i - 2] + WA)
        return slots + [slots[-1] + 1, slots[-1] + 2], emit

    def st_halo(t, kv, slots):
        dst, src = BUF[t % 2][kv], BUF[1 - t % 2][kv]

        def emit(j, tk):
            sub = lax.broadcasted_iota(i32, (8, 128), 0) | pltpu.bitcast(tk(), i32)
            for m in range(1, HV + 1):
                a0 = (HV + NG - m) * 8
                if t == 0:
                    top = 0.0
                else:
                    top = src[j, a0 + 7:a0 + 15, :]
                    if t == 1 and kv == 2:
                        top = top + bias_v[NJ + j]
                dst[j, (HV - m) * 8:(HV - m + 1) * 8, :] = jnp.where(sub < 1, top, dst[j, a0 - 1:a0 + 7, :])
        return slots, emit

    def st_ln1(t, slots, fin, mo):
        h_r, row0 = BUF[t % 2][0], t * TM
        l1, hs = {}, {}
        order = [2 * (4 * i + m) + p for m in mo for i in range(4) for p in range(2)]

        def ldx(g, z):
            r = 64 * (g // 8) + 8 * ((g // 2) % 4) + 32 * (g % 2)
            return [x_3[z, pl.ds(row0 + r, 8), j * 128:(j + 1) * 128].astype(f32) for j in range(NJ)]

        def n1(g, tok):
            xf = ldx(g, 0)
            xf[0] = xf[0] + pltpu.bitcast(tok, f32)
            l1[g] = (lsum(tree(xf)), lsum(tree([x * x for x in xf])))

        def n3(g, dl):
            m, rs = stats(*l1.pop(g))
            xf = ldx(g, zs[0])
            hs[g] = [(xf[j] - m) * rs * mrow(1, j) + mrow(0, j) for j in range(NJ)]
            if g % 2 == 1:
                b = g // 2
                h0 = hs.pop(g - 1)
                h1 = hs.pop(g)
                pk = [pack2(h0[j], h1[j]) for j in range(NJ)]
                for j in range(NJ):
                    h_r[j, pl.ds(32 * (b % 4) + b // 4, 8, stride=4), :] = pk[j]
                fin(dl, orall(pk))

        def emit(i, tk):
            if i < NG:
                n1(order[i], tk())
            if 0 <= i - 1 < NG:
                n3(order[i - 1], slots[i - 1] + WL)
        return slots + [slots[-1] + 1], emit

    def st_apply(t, slots, fin):
        order = sorted(range(NG // 2), key=lambda b: b % 4)

        def emit(i, tk):
            b = order[i]
            r = t * TM + 64 * (b // 4) + 8 * (b % 4)
            pk = [pack2(h2_v[r:r + 8, j * 128:(j + 1) * 128] * mrow(1, j),
                        h2_v[r + 32:r + 40, j * 128:(j + 1) * 128] * mrow(1, j)) for j in range(NJ)]
            for j in range(NJ):
                BUF[t][0][j, pl.ds(32 * (b % 4) + b // 4, 8, stride=4), :] = pk[j]
            if fin is not None:
                fin(slots[i] + 3, orall(pk))
        return slots, emit

    def st_post(t, slots, fin, mo, end, snap=None):
        x1_rs, row0 = x1s[4 * (t % 2):4 * (t % 2) + 4], t * TM
        p1s, p3s, bst, ends = {}, {}, {}, []
        order = [4 * ci + m for m in mo for ci in range(GM)]

        def ldx1(g, z):
            return [x1_rs[g % 4][j, pl.ds((g // 4) * 8 + zo(z), 8), :] for j in range(NJ)]

        def p1(g, tok):
            xf = ldx1(g, 0)
            if tok is not None:
                xf[0] = xf[0] + pltpu.bitcast(tok, f32)
            p1s[g] = (lsum(tree(xf)), lsum(tree([x * x for x in xf])))

        def p3(g, dl):
            x1 = ldx1(g, 1)
            m, rs = stats(*p1s.pop(g))
            nn = [(x1[j] - m) * rs for j in range(NJ)]
            ov = [(x1[j] + mrow(7, j)) + nn[j] * mrow(6, j) for j in range(NJ)]
            p3s[g] = lsum(tree([nn[j] * mrow(8, j) for j in range(NJ)]))
            h2_v[pl.ds(row0 + g * 8, 8), :] = jnp.concatenate(nn, axis=1)
            out_v[pl.ds(row0 + g * 8, 8), :] = jnp.concatenate(ov, axis=1).astype(bf16)
            ends.append(orall([pltpu.bitcast(o, u32) for o in ov[PT:]]))
            fin(dl, ends[-1])

        def p4(g, n, dl):
            rg = (p3s.pop(g) + mrow(9, 0)).astype(bf16).astype(f32)
            m = g % 4
            if n % GM == 0:
                bst['v'] = best_v[m * 8:(m + 1) * 8, :]
                bst['i'] = besti_v[m * 8:(m + 1) * 8, :]
            upd = rg > bst['v']
            bst['v'] = jnp.where(upd, rg, bst['v'])
            bst['i'] = jnp.where(upd, row0 + g * 8, bst['i'])
            if n % GM == GM - 1:
                best_v[m * 8:(m + 1) * 8, :] = bst['v']
                besti_v[m * 8:(m + 1) * 8, :] = bst['i']
            if n % 2 == 1:
                fin(dl, pltpu.bitcast(bst['i'], u32))

        def emit(i, tk):
            if i < NG:
                p1(order[i], tk())
            if 0 <= i - 1 < NG:
                p3(order[i - 1], slots[i - 1] + WP)
            if 0 <= i - 2 < NG:
                p4(order[i - 2], i - 2, slots[i - 2] + WP + 2)
            if snap is not None and i - 2 == SNAP * GM - 1:
                snap()
            if i == NG:
                end()
                if snap is not None:
                    spec.append(orall(ends[SNAP * GM:]))
        return slots + [slots[-1] + 1, slots[-1] + 2], emit

    def st_perm(t, js, slots, fin, dl):
        cst = {}

        def emit(r, tk):
            if r == 0:
                lane = lax.broadcasted_iota(i32, (8, 128), 1)
                cls = (lane // 4) % 5
                cst['m'] = [cls == c for c in range(1, NJ)]
                for j in js:
                    cst[j] = 4 * ((5 * (lane % 32) + j) % 32) + lane // 32
            srcs = [tou(wqkv_raw[r * 16:(r + 1) * 16, t * D + i * 128:t * D + (i + 1) * 128]) for i in range(NJ)]
            for j in js:
                m = srcs[(j * 3) % 5]
                for c in range(1, NJ):
                    m = jnp.where(cst['m'][c - 1], srcs[((j + 5 - c) * 3) % 5], m)
                m = jnp.take_along_axis(m, cst[j], axis=1)
                wq_p[t * NJ + j][r * 8:(r + 1) * 8, :] = m
            if fin is not None:
                fin(slots[r] + dl, m)
        return slots, emit

    def st_perm_o(slots, fin, dl):
        def emit(i, tk):
            n, j = (i % 25) // NJ, i % NJ
            if i < 25:
                w = wo_raw[j * 128:(j + 1) * 128, n * 128:(n + 1) * 128].astype(f32) * (
                    mrow(2, n) + pltpu.bitcast(tk(), f32))[0:1]
                wo_f[n, j * 128:(j + 1) * 128, :] = w
                fin(slots[i] + dl, pltpu.bitcast(w[120:128], u32))
                return
            for dd in range(4):
                for hh in range(2):
                    r0 = hh * 16 * DH + 4 * j + dd
                    ev = wo_f[n, pl.ds(r0, 8, stride=2 * DH), :]
                    od = wo_f[n, pl.ds(r0 + DH, 8, stride=2 * DH), :]
                    p0 = j * 64 + dd * 16 + hh * 8
                    pk = pack2(ev, od)
                    wo_p[n][p0:p0 + 8, :] = pk
            fin(slots[i] + dl, pk)
        return slots, emit

    class Phase:
        def __init__(self, carry=None):
            self.done = {}
            self.tok = None
            if carry is not None:
                self.done = dict(carry.left)
                self.tok = carry.tok
            self.cur = 0

        def fin(self, slot, v):
            self.done.setdefault(max(slot, self.cur), []).append(v)

        def run(self, jobs, streams):
            pos = [0] * len(streams)
            pend = []
            for c in range(len(jobs) + 1):
                self.cur = c
                cache = []

                def tk():
                    if self.tok is None:
                        return None
                    if not cache:
                        cache.append(zand(self.tok))
                    return cache[0]
                for si, (slots, emit) in enumerate(streams):
                    while pos[si] < len(slots) and (slots[pos[si]] <= c or c == len(jobs)):
                        emit(pos[si], tk)
                        pos[si] += 1
                if c == len(jobs):
                    break
                pend += self.done.pop(c, [])
                r = jobs[c](pend)
                if r is not None:
                    self.tok = r
                    pend = []
            self.left = {k - len(jobs): v for k, v in self.done.items()}

    def out_cp(t):
        return pltpu.make_async_copy(out_v.at[pl.ds(t * TM, TM)], out_hbm.at[pl.ds(t * TM, TM)], sems.at[10])

    best_v[...] = jnp.full((32, 128), -jnp.inf, f32)
    besti_v[...] = jnp.zeros((32, 128), i32)
    for r_ in (ka, kb, va, vb):
        for j in range(NJ):
            r_[j, KVR - 8:KVR, :] = jnp.zeros((8, 128), f32)
    wait(g_z)
    zv = pltpu.bitcast(zero_v[...], i32)
    for i in range(4):
        zs[i] = zv[i, 0]
    wait(g_x0)
    cf = c_v[...].astype(f32)
    sc_v[...] = tou(jnp.broadcast_to((cf * jax.nn.sigmoid(cf)).astype(bf16), (16, D)))
    for g in range(2 * NG):
        xf = [x_v[g * 8:(g + 1) * 8, j * 128:(j + 1) * 128].astype(f32) for j in range(NJ)]
        m_, rs_ = stats(lsum(tree(xf)), lsum(tree([x * x for x in xf])))
        h2_v[g * 8:(g + 1) * 8, :] = jnp.concatenate([(x - m_) * rs_ for x in xf], axis=1)
    wait(g_wq)
    Phase().run([], [st_perm(0, [j], [0] * 40, None, 0) for j in range(NJ)])
    wait(g_ca)
    for j in range(NJ):
        job_mod(1, j)([])

    ph = Phase()
    fin = ph.fin
    mo = [2, 3, 0, 1]
    nat = list(range(NM))
    jobs, streams, spec = [], [], []

    def nmaj(t, ns, bias=False):
        return [job_qkv(t, n, m, (1 if m == 0 else 2) if bias == 1 else bias) for n in ns for m in nat]

    def mmaj(t, ns):
        return [job_qkv(t, n, m) for m in mo for n in ns]

    def waiter(g, *keys):
        def f():
            wait(g)
        return job_call(f)

    QS, KS, VS = range(NJ), range(NJ, 2 * NJ), range(2 * NJ, 3 * NJ)
    K3 = 24; K5 = 4; K4 = 18
    jobs += nmaj(0, QS) + nmaj(1, QS) + nmaj(0, KS)
    jobs.insert(60 - K5, waiter(g_wv, ('raw', 2)))
    for j in range(NJ):
        jobs.insert(60 - K5 + 1 + j, job_mod(0, j))
    jobs.insert(K3, waiter(g_wk, ('raw', 1)))
    s5 = 62 - K5
    sv0 = len(jobs)
    for j in range(NJ):
        jobs += nmaj(0, [2 * NJ + j], 1) + [job_bq(j)]
    sk1 = len(jobs)
    jobs += nmaj(1, KS, 1)
    sv1 = len(jobs)
    jobs += nmaj(1, VS, 2)
    jobs.insert(len(jobs) - K4, waiter(g_xr, 'x'))
    s4 = len(jobs) - K4
    streams += [st_apply(0, [0] * 16, None), st_apply(1, _spread(16, 2, 16), fin)]
    streams += [st_perm(1, [j], _spread(40, K3 + 1 + 5 * j, K3 + 5 + 5 * j), fin, 2) for j in range(NJ)]
    streams += [st_perm(2, [j], _spread(40, s5, s5 + NJ + K5 - 1) if j == 0 else
                        _spread(40, sv0 + 5 * j - 6, sv0 + 5 * j - 2), fin, 1) for j in range(NJ)]
    st = {}
    for t in range(2, NT):
        if t == 6:
            jobs.append(waiter(g_rest))
        st[t] = len(jobs)
        jl = mmaj(t, QS) + nmaj(t, KS) + nmaj(t, VS) if t < NT - 1 else mmaj(t, KS) + nmaj(t, VS) + mmaj(t, QS)
        for i, jb in enumerate(jl):
            jobs.append(jb)
            if t == 6 and i % 3 == 1:
                jobs.append(job_mod(2 + (i // 3) // NJ, (i // 3) % NJ))

    def consts():
        cb, sb, gbv = mod_v[:, 4 * D:5 * D], mod_v[:, 3 * D:4 * D], mod_v[:, 5 * D:6 * D]
        wr = jnp.broadcast_to(wr_v[...].astype(f32).reshape(1, D), (8, D))
        mod_v[:, 6 * D:7 * D] = gbv * cb
        mod_v[:, 7 * D:8 * D] = gbv * sb
        mod_v[:, 8 * D:9 * D] = cb * wr
        mod_v[:, 9 * D:9 * D + 128] = jnp.broadcast_to(lsum(sb * wr), (8, 128))

    jobs.insert(st[7] + 20, job_call(consts))
    f6, f7 = st[7], len(jobs)

    def argmax(row):
        bv = best_v[...]
        bi = besti_v[...] + (lax.broadcasted_iota(i32, (32, 128), 0) & 7)
        mx = jnp.max(bv, axis=0, keepdims=True)
        cand = jnp.where(bv == mx, bi, S)
        idxv = jnp.min(cand, axis=0, keepdims=True)
        idx = jnp.minimum(idxv, S - 1)[0, 0]
        return mx, idx, h2_v[pl.ds(idx, 1), :] if row else None

    def gap(n, lo, hi, bar, taper):
        return [x if x < bar - taper else x + taper + 1 for x in _spread(n, lo, hi - taper - 1)]

    TP = 5; AX = 10; AY = 3; LX = 8
    streams += [st_halo(0, 2, _spread(NJ, sv0 + 4, sv0 + 20)), st_halo(0, 3, _spread(NJ, sk1 + 4, sk1 + 14)),
                st_halo(1, 2, _spread(NJ, s4 + 4, s4 + 14)), st_halo(1, 3, _spread(NJ, st[2] + 4, st[2] + 16))]
    for t in range(2, NT - 1):
        streams += [st_halo(t, 2, _spread(NJ, st[t + 1] - 16, st[t + 1] - 6)),
                    st_halo(t, 3, _spread(NJ, st[t + 1] + 4, st[t + 1] + 16))]
    streams += [st_halo(7, 2, _spread(NJ, f6 + 28, f6 + 42)), st_halo(7, 3, _spread(NJ, f6 + 48, f6 + 60))]
    a_lo = [sk1 + 2, st[2] + AX, st[3] + AX - AY, st[4] + AX - 2 * AY, st[5] + max(AX - 3 * AY, 1)]
    streams.append(st_attention(0, gap(NG, a_lo[0], a_lo[1], s4 - 1, TP), fin))
    for t in range(1, 4):
        streams.append(st_attention(t, _spread(NG, a_lo[t], a_lo[t + 1]), fin))
    streams.append(st_attention(4, _spread(NG, a_lo[4], st[6] - ATHI), fin))
    T0 = 0; T1 = 46; T2 = 48; T3 = 136; T4 = 10; T5 = 8
    streams.append(st_attention(5, _spread(NG, st[6], f6 + T0), fin))
    streams.append(st_attention(6, _spread(NG, f6 + max(T0, 1), f6 + T1), fin))
    streams.append(st_attention(7, _spread(T4, f6 + T2, f7 + T5) + _spread(NG - T4, f7 + T5, f7 + T3), fin,
                                order=[(i + 16) % NG for i in range(NG)]))
    streams.append(st_ln1(2, _spread(NG, s4, st[2] + LX), fin, mo))
    for t in range(3, 6):
        streams.append(st_ln1(t, _spread(NG, st[t - 1] + LX, st[t] + LX), fin, mo))
    streams.append(st_ln1(6, _spread(NG, st[5] + LX, st[6] - LNHI), fin, mo))
    streams.append(st_ln1(7, _spread(NG, st[6], st[7] + 0), fin, mo))
    streams.append(st_perm_o(_spread(25, f6 + 4, f6 + 24) + _spread(25, f6 + 26, f6 + 54), fin, 4))
    for t in range(NT):
        mt = mo if t == NT - 1 else nat
        jobs += [job_wo(t, c, m) for m in mt for c in range(NJ)]
        s0 = f7 + 20 * t + POLO
        sl = _spread(NG, s0, s0 + 20)
        if t == NT - 1:
            sl = [min(sl[i], s0 - POLO + PL7 + 5 * (i // 8) + (i % 8) // 3) for i in range(NG)]
        streams.append(st_post(t, sl, fin, mt, out_cp(t).start,
                               (lambda: spec.append(argmax(True))) if t == NT - 1 else None))
    ph.run(jobs, streams)

    def moe(mx, idx, nrow, after=None):
        base = pl.multiple_of((idx // 16) * 16, 16)
        hrow = jnp.broadcast_to(nrow, (8, D)) * mod_v[:, 4 * D:5 * D] + mod_v[:, 3 * D:4 * D]
        hrow = hrow.astype(bf16).astype(f32)
        hf = [hrow[:, j * 128:(j + 1) * 128] for j in range(NJ)]
        h16 = [tob(pack2(h, h)) for h in hf]
        NC = 7
        NV = (F - NC * 128) // 8

        def glu(g, u):
            hg = 0.5 * g
            return (hg * jnp.tanh(hg) + hg) * u

        def ntdot(w_v, c):
            return tree([lax.dot_general(h16[j], w_v[c * 128:(c + 1) * 128, j * 128:(j + 1) * 128],
                                         (((1,), (1,)), ((), ())),
                                         preferred_element_type=f32)[0:8] for j in range(NJ)])

        def wrow(w_v, r0, j):
            return w_v[r0:r0 + 8, j * 128:(j + 1) * 128].astype(f32)

        ym, acts, acc, toks = None, [], None, []
        MD = 2
        MA = 3
        NP = 2 * NC - 1 + MD
        for c in range(2 * NC + 2):
            if c < 2 * NC:
                toks.append(ntdot(wu_v if c % 2 else wg_v, c // 2))
                if c % 2:
                    a8 = glu(toks[c - 1], toks[c])
                    acts.append(tob(pack2(a8, a8)))
            if c > 2 and c % 2:
                k = (c - 3) // 2
                yc = [jnp.dot(acts[k], wd_v[k * 128:(k + 1) * 128, j * 128:(j + 1) * 128],
                              preferred_element_type=f32)[0:8] for j in range(NJ)]
                ym = yc if ym is None else [ym[j] + yc[j] for j in range(NJ)]
            if c < NP:
                tk_ = None if c < MD else pltpu.bitcast(toks[c - MD], u32)
                if after is not None and c == MA:
                    tk_ = after if tk_ is None else tk_ | after
                h0 = hf if tk_ is None else [h + pltpu.bitcast(zand(tk_), f32) for h in hf]
                for i in range(c * NV // NP, (c + 1) * NV // NP):
                    r0 = NC * 128 + i * 8
                    g = lsum(tree([wrow(wg_v, r0, j) * h0[j] for j in range(NJ)]))
                    u = lsum(tree([wrow(wu_v, r0, j) * h0[j] for j in range(NJ)]))
                    av = glu(g, u)
                    pr = [wrow(wd_v, r0, j) * av for j in range(NJ)]
                    acc = pr if acc is None else [acc[j] + pr[j] for j in range(NJ)]
        y = jnp.concatenate(ym, axis=1)[0:1] + jnp.sum(jnp.concatenate(acc, axis=1), axis=0, keepdims=True)
        y = y * jax.nn.sigmoid(mx[:, 0:1])
        rows = base + lax.broadcasted_iota(i32, (16, D), 0)
        gb = mod_v[0:1, 5 * D:6 * D]
        old = out_v[pl.ds(base, 16), :].astype(f32)
        newblk = jnp.where(rows == idx, old + gb * y, old)
        fix_v[...] = newblk.astype(bf16)

    moe(*spec[0], spec[1])
    mx_f, idx_f, _ = argmax(False)
    for t in range(NT):
        out_cp(t).wait()

    @pl.when(idx_f != spec[0][1])
    def _():
        moe(mx_f, idx_f, h2_v[pl.ds(idx_f, 1), :])

    base_f = pl.multiple_of((idx_f // 16) * 16, 16)
    fix = pltpu.make_async_copy(fix_v, out_hbm.at[pl.ds(base_f, 16)], sems.at[0])
    fix.start()
    fix.wait()


@jax.jit
def pallas_adaLN_cond__sliding_local_dilated__moe_arch_mod__prompt_kernel(
    A_x, A_wqkv, A_wo, B_x, B_w_r, B_w_gate, B_w_up, B_w_down, c, w_mod,
):
    x = A_x.reshape(S, D)
    V = pltpu.VMEM
    scratch = [V((D // 2, 128), u32)] * 20 + [V((NJ, MS, 128), f32)] * 8 + [
        V((1, S, D), bf16),
        V((3 * NJ + 1, 8, 128), f32),
        V((D, 3 * D), bf16),
        V((D, D), bf16),
        V((NJ, D, 128), f32),
        V((F, D), bf16),
        V((F, D), bf16),
        V((F, D), bf16),
        V((D, 6 * D), bf16),
        V((8, 9 * D + 128), f32),
        V((NJ, TM // 2, 128), u32), V((NJ, TM // 2, 128), u32),
        V((NJ, TM, 128), f32), V((NJ, TM, 128), f32),
        V((NJ, KVR, 128), f32), V((NJ, KVR, 128), f32),
        V((NJ, KVR, 128), f32), V((NJ, KVR, 128), f32),
        V((NT - 1, NJ, TM // 2, 128), u32), V((NJ, TM // 2, 128), u32),
        V((S, D), f32),
        V((S, D), bf16),
        V((32, 128), f32),
        V((32, 128), i32),
        V((8, 128), u32),
        V((8, 128), u32),
        V((8, D), u32),
        V((8, D), u32),
        V((16, D), bf16),
        V((1, D), bf16),
        V((D,), bf16),
        pltpu.SMEM((4,), i32),
        pltpu.SemaphoreType.DMA((NSEM,)),
    ]
    out = pl.pallas_call(
        _kernel,
        out_shape=jax.ShapeDtypeStruct((S, D), bf16),
        in_specs=[pl.BlockSpec(memory_space=pltpu.HBM)] * 9,
        out_specs=pl.BlockSpec(memory_space=pltpu.HBM),
        scratch_shapes=scratch,
        compiler_params=pltpu.CompilerParams(vmem_limit_bytes=100 * 2**20),
    )(x, A_wqkv, A_wo, B_w_r, B_w_gate.T, B_w_up.T, B_w_down, c, w_mod)
    return out.reshape(1, S, D)
```

```python
import math

import jax
import jax.numpy as jnp
from jax import lax
import jax.experimental.pallas as pl
import jax.experimental.pallas.tpu as pltpu


S = 2048
D = 640
H = 32
DH = 20
WIN = 8
F = 1728
NJ = D // 128
TM = 256
NT = S // TM
NG = TM // 8
HV = 14
MS = 64
NM = TM // MS
GM = MS // 8
KVR = (HV + NG + 1) * 8
EPS = 1e-5
LOG2E = math.log2(math.e)
QSCALE = (DH ** -0.5) * LOG2E
NEG = -1000000000.0 * LOG2E
f32 = jnp.float32
bf16 = jnp.bfloat16
u32 = jnp.uint32
i32 = jnp.int32
KL = 3
QLO = 8 * KL
NSEM = 12

WA = 20
WL = 16
WP = 11
CH = 2
ATHI = 8
LNHI = 4
POLO = 7
PL7 = 6
PT = 2
SNAP = 2
WA2 = 16
WA3 = 16
FA = 5
FL = 5


def _spread(n, lo, hi):
    return [int(lo + (i * (hi - lo)) / n) for i in range(n)]


def _kernel(x_hbm, wqkv_hbm, wo_hbm, wr_hbm, wg_hbm, wu_hbm, wd_hbm, c_hbm, wmod_hbm,
            out_hbm, *wp):
    (x_3, bias_v, wqkv_raw, wo_raw, wo_f, wg_v, wu_v, wd_v, wmod_v,
     mod_v, ha, hb, hc, qa, qb, qc, ka, kb, kc, va, vb, vc, o_all, oc, h2_v, out_v, best_v, besti_v,
     zsrc, zero_v, sc_v, sap_v, fix_v, c_v, wr_v, zs, sems) = wp[28:]
    x_v = x_3.at[0]
    wq_p = wp[:15]
    wo_p = wp[15:20]
    x1s = wp[20:28]

    def cp(src, dst, i):
        n = src.shape[0]
        if n < 64 or not 0:
            return [(pltpu.make_async_copy(src, dst, sems.at[i]), 0)]
        return [(pltpu.make_async_copy(src.at[pl.ds(p * n // 2, n // 2)], dst.at[pl.ds(p * n // 2, n // 2)],
                                       sems.at[i]), p * 0) for p in range(2)]

    def xcp(t0, nt, i):
        return cp(x_hbm.at[pl.ds(t0 * TM, nt * TM)], x_v.at[pl.ds(t0 * TM, nt * TM)], i)

    def colcp(src, dst, k0, nk, i, r0=0, nr=D):
        return cp(src.at[pl.ds(r0, nr), pl.ds(k0 * D, nk * D)], dst.at[pl.ds(r0, nr), pl.ds(k0 * D, nk * D)], i)

    def wait(g):
        for d, _ in g:
            d.wait()

    g_z = cp(zsrc, zero_v, 0)
    g_x0 = xcp(0, 1, 1) + cp(c_hbm, c_v, 1)
    g_wq = colcp(wqkv_hbm, wqkv_raw, 0, 1, 2, 0, 16 * QLO)
    g_wq2 = colcp(wqkv_hbm, wqkv_raw, 0, 1, 10, 16 * QLO, D - 16 * QLO) + xcp(1, 1, 10)
    g_ca = colcp(wmod_hbm, wmod_v, 1, 1, 3)
    g_wk = colcp(wqkv_hbm, wqkv_raw, 1, 1, 4)
    g_wv = colcp(wqkv_hbm, wqkv_raw, 2, 1, 5) + colcp(wmod_hbm, wmod_v, 0, 1, 5) + xcp(2, 1, 5)
    g_xr = xcp(3, 5, 6)
    g_rest = (colcp(wmod_hbm, wmod_v, 2, 4, 7) + cp(wo_hbm, wo_raw, 11) + [(pltpu.make_async_copy(wr_hbm, wr_v, sems.at[11]), 0)]
              + cp(wg_hbm, wg_v, 8) + cp(wu_hbm, wu_v, 9) + cp(wd_hbm, wd_v, 11))
    zsrc[...] = jnp.zeros((8, 128), u32)
    for d, p in g_x0 + g_ca + g_wq + g_wq2 + g_z + g_wk + g_wv + g_xr + g_rest:
        d.start(priority=p)

    BUF = [(ha, qa, ka, va), (hb, qb, kb, vb), (hc, qc, kc, vc)]

    def tob(u):
        return pltpu.bitcast(u, bf16)

    def tou(b):
        return pltpu.bitcast(b, u32)

    def pack2(a, b):
        return pltpu.bitcast(pltpu.pack_elementwise([a, b], packed_dtype=bf16), u32)

    def zand(v):
        return pltpu.bitcast(v, u32) & zero_v[...]

    def orall(vs):
        r = vs[0]
        for v in vs[1:]:
            r = r | v
        return r

    def mrow(k, j):
        return mod_v[:, k * D + j * 128:k * D + (j + 1) * 128]

    def tree(vs):
        return ((vs[0] + vs[1]) + (vs[2] + vs[3])) + vs[4]

    def lsum(v):
        return jnp.sum(v, axis=-1, keepdims=True)

    def stats(s, s2):
        m = s * (1.0 / D)
        v = jnp.maximum(s2 * (1.0 / D) - m * m, 0.0)
        return m, jnp.exp2(jnp.log(v + EPS) * (-0.5 * LOG2E))

    def zo(i):
        return pl.multiple_of(zs[i], 8)

    def oref(t):
        return oc if t == NT - 1 else o_all.at[t]

    def gated(w, toks):
        if toks:
            t = orall(toks) & zero_v[...]
            w = jnp.concatenate([w[0:8] | t, w[8:]], axis=0)
        return tob(w)

    def lhs(ref, m, extra=None):
        a = jnp.concatenate([ref[j, m * MS // 2:(m + 1) * MS // 2] for j in range(NJ)], axis=1)
        if extra is not None:
            a = jnp.concatenate([a, extra], axis=0)
        return tob(a)

    def job_qkv(t, n, m, bias=0):
        h_r, q_r, k_r, v_r = BUF[t % 3]

        def run(toks):
            res = jnp.dot(lhs(h_r, m, sap_v[...] if bias == 1 else None),
                          gated(wq_p[n][pl.ds(zo(m), D // 2), :], toks),
                          preferred_element_type=f32)
            if bias:
                if bias == 1:
                    bb = res[MS:MS + 8]
                    bias_v[n] = bb
                else:
                    bb = bias_v[n, pl.ds(zo(m), 8), :]
                res = jnp.concatenate([res[i * 8:(i + 1) * 8] + bb for i in range(GM)], axis=0)
            if n < NJ:
                q_r[n, m * MS:(m + 1) * MS, :] = res
            elif n < 2 * NJ:
                k_r[n - NJ, HV * 8 + m * MS:HV * 8 + (m + 1) * MS, :] = res
            else:
                v_r[n - 2 * NJ, HV * 8 + m * MS:HV * 8 + (m + 1) * MS, :] = res
            return res[0:8]
        return run

    def job_q0(n, m, hi):
        js = range(KL, NJ) if hi else range(KL)

        def run(toks):
            a = jnp.concatenate([ha[j, m * MS // 2:(m + 1) * MS // 2] for j in js], axis=1)
            res = jnp.dot(tob(a), gated(wq_p[n][pl.ds(js[0] * 64 + zo(m), len(js) * 64), :], toks),
                          preferred_element_type=f32)
            if hi:
                res = res + qa[n, m * MS:(m + 1) * MS, :]
            qa[n, m * MS:(m + 1) * MS, :] = res
            return res[0:8]
        return run

    def job_bq(n):
        def run(toks):
            bias_v[n] = jnp.dot(tob(sap_v[...]), tob(wq_p[n][pl.ds(zo(0), D // 2), :]),
                                preferred_element_type=f32)[0:8]
            return None
        return run

    def job_wo(t, c, m):
        o_r, x1_r, row0 = oref(t), x1s[4 * (t % 2) + m], t * TM

        def run(toks):
            a = jnp.dot(lhs(o_r, m), gated(wo_p[c][pl.ds(zo(m), D // 2), :], toks),
                        preferred_element_type=f32)
            for ci in range(GM):
                cc = m * GM + ci
                g = 4 * (cc % 8) + cc // 8
                xr = x_v[pl.ds(row0 + g * 8, 8), c * 128:(c + 1) * 128].astype(f32)
                x1_r[c, ci * 8:(ci + 1) * 8, :] = xr + a[ci * 8:(ci + 1) * 8]
            return a[0:8]
        return run

    def job_mod(k, j):
        def run(toks):
            lo = k * D + j * 128
            m = jnp.dot(tob(sc_v[...]), wmod_v[:, lo:lo + 128], preferred_element_type=f32).astype(bf16)
            if k == 0:
                sap_v[:, j * 128:(j + 1) * 128] = tou(m)
            m = m[:8].astype(f32)
            if k in (1, 4):
                m = m + 1.0
            mod_v[:, lo:lo + 128] = m
            return None
        return run

    def job_call(fn):
        def run(toks):
            fn()
            return None
        return run

    def st_attention(t, slots, fin, order=None):
        _, q_c, k_c, v_c = BUF[t % 3]
        o_c = oref(t)
        first = t == 0
        st1, st2, outs, chain = {}, {}, {}, []
        order = order or [(i + HV) % NG for i in range(NG)]

        def ld(ref, j, i):
            return ref[j, (HV + i) * 8:(HV + i + 1) * 8, :]

        def a1(g, tok):
            if CH and len(chain) >= CH:
                ct = zand(chain[-CH])
                tok = ct if tok is None else tok | ct
            sc = QSCALE if tok is None else pltpu.bitcast(
                pltpu.bitcast(jnp.full((8, 128), QSCALE, f32), u32) | tok, f32)
            if t < 2:
                q = [(q_c[j, g * 8:(g + 1) * 8, :] + bias_v[j, pl.ds(zo(0), 8), :]) * sc for j in range(NJ)]
            else:
                q = [q_c[j, g * 8:(g + 1) * 8, :] * sc for j in range(NJ)]
            ps = []
            for w in range(WIN):
                p = q[0] * ld(k_c, 0, g - 2 * w)
                for j in range(1, NJ):
                    p = p + q[j] * ld(k_c, j, g - 2 * w)
                ps.append((p, pltpu.roll(p, 64, 1)))
            st1[g] = ps

        def a2(g):
            ps = []
            for (p, pr) in st1.pop(g):
                p = p + pr
                ps.append((p, pltpu.roll(p, 32, 1)))
            st2[g] = ps

        def a3(g, dl):
            ls = [p + pr for (p, pr) in st2.pop(g)]
            if first:
                sub = lax.broadcasted_iota(i32, (8, 128), 0)
                ls = [jnp.where(sub > 0, ls[w], NEG) if g - 2 * w < 0 else ls[w] for w in range(WIN)]
            m = jnp.maximum(jnp.maximum(jnp.maximum(ls[0], ls[1]), jnp.maximum(ls[2], ls[3])),
                            jnp.maximum(jnp.maximum(ls[4], ls[5]), jnp.maximum(ls[6], ls[7])))
            es = [jnp.exp2(l - m) for l in ls]
            den = ((es[0] + es[1]) + (es[2] + es[3])) + ((es[4] + es[5]) + (es[6] + es[7]))
            inv = pl.reciprocal(den, approx=True)
            o = []
            for j in range(NJ):
                acc = es[0] * ld(v_c, j, g)
                for w in range(1, WIN):
                    acc = acc + es[w] * ld(v_c, j, g - 2 * w)
                o.append(acc * inv)
            outs[g] = o
            chain.append(o[NJ - 1])
            if g % 2 == 1:
                o0 = outs.pop(g - 1)
                o1 = outs.pop(g)
                pk = [pack2(o0[j], o1[j]) for j in range(NJ)]
                for j in range(NJ):
                    o_c[j, pl.ds(32 * (g // 8) + (g // 2) % 4, 8, stride=4), :] = pk[j]
                if FA:
                    fin(dl, orall(pk[NJ - FA:]))

        def emit(i, tk):
            if i < NG:
                a1(order[i], tk())
            if 0 <= i - 1 < NG:
                a2(order[i - 1])
            if 0 <= i - 2 < NG:
                a3(order[i - 2], slots[i - 2] + (WA if t < 5 else WA2 if t < 7 else WA3))
        return slots + [slots[-1] + 1, slots[-1] + 2], emit

    def st_halo(t, kv, slots):
        dst, src = BUF[t % 3][kv], BUF[(t - 1) % 3][kv]

        def emit(j, tk):
            sub = lax.broadcasted_iota(i32, (8, 128), 0) | pltpu.bitcast(tk(), i32)
            for m in range(1, HV + 1):
                a0 = (HV + NG - m) * 8
                if t == 0:
                    top = 0.0
                else:
                    top = src[j, a0 + 7:a0 + 15, :]
                    if t == 2 and kv == 2:
                        top = top + bias_v[NJ + j]
                dst[j, (HV - m) * 8:(HV - m + 1) * 8, :] = jnp.where(sub < 1, top, dst[j, a0 - 1:a0 + 7, :])
        return slots, emit

    def st_ln1(t, slots, fin, mo):
        h_r, row0 = BUF[t % 3][0], t * TM
        l1, hs = {}, {}
        order = [2 * (4 * i + m) + p for m in mo for i in range(4) for p in range(2)]

        def ldx(g, z):
            r = 64 * (g // 8) + 8 * ((g // 2) % 4) + 32 * (g % 2)
            return [x_3[z, pl.ds(row0 + r, 8), j * 128:(j + 1) * 128].astype(f32) for j in range(NJ)]

        def n1(g, tok):
            xf = ldx(g, 0)
            xf[0] = xf[0] + pltpu.bitcast(tok, f32)
            l1[g] = (lsum(tree(xf)), lsum(tree([x * x for x in xf])))

        def n3(g, dl):
            m, rs = stats(*l1.pop(g))
            xf = ldx(g, zs[0])
            hs[g] = [(xf[j] - m) * rs * mrow(1, j) for j in range(NJ)]
            if t > 1:
                hs[g] = [hs[g][j] + mrow(0, j) for j in range(NJ)]
            if g % 2 == 1:
                b = g // 2
                h0 = hs.pop(g - 1)
                h1 = hs.pop(g)
                pk = [pack2(h0[j], h1[j]) for j in range(NJ)]
                for j in range(NJ):
                    h_r[j, pl.ds(32 * (b % 4) + b // 4, 8, stride=4), :] = pk[j]
                if FL:
                    fin(dl, orall(pk[NJ - FL:]))

        def emit(i, tk):
            if i < NG:
                n1(order[i], tk())
            if 0 <= i - 1 < NG:
                n3(order[i - 1], slots[i - 1] + (WL if t > 1 else 20 if i < 12 else 8))
        return slots + [slots[-1] + 1], emit

    def st_apply(t, slots, fin):
        order = sorted(range(NG // 2), key=lambda b: b % 4)

        def emit(i, tk):
            b = order[i]
            r = t * TM + 64 * (b // 4) + 8 * (b % 4)
            pk = [pack2(h2_v[r:r + 8, j * 128:(j + 1) * 128] * mrow(1, j),
                        h2_v[r + 32:r + 40, j * 128:(j + 1) * 128] * mrow(1, j)) for j in range(NJ)]
            for j in range(NJ):
                BUF[t][0][j, pl.ds(32 * (b % 4) + b // 4, 8, stride=4), :] = pk[j]
            if fin is not None:
                fin(slots[i] + 3, orall(pk))
        return slots, emit

    def st_post(t, slots, fin, mo, end, snap=None):
        x1_rs, row0 = x1s[4 * (t % 2):4 * (t % 2) + 4], t * TM
        p1s, p3s, bst, ends = {}, {}, {}, []
        order = [4 * ci + m for m in mo for ci in range(GM)]

        def ldx1(g, z):
            return [x1_rs[g % 4][j, pl.ds((g // 4) * 8 + zo(z), 8), :] for j in range(NJ)]

        def p1(g, tok):
            xf = ldx1(g, 0)
            if tok is not None:
                xf[0] = xf[0] + pltpu.bitcast(tok, f32)
            p1s[g] = (lsum(tree(xf)), lsum(tree([x * x for x in xf])))

        def p3(g, dl):
            x1 = ldx1(g, 1)
            m, rs = stats(*p1s.pop(g))
            nn = [(x1[j] - m) * rs for j in range(NJ)]
            ov = [(x1[j] + mrow(7, j)) + nn[j] * mrow(6, j) for j in range(NJ)]
            p3s[g] = lsum(tree([nn[j] * mrow(8, j) for j in range(NJ)]))
            h2_v[pl.ds(row0 + g * 8, 8), :] = jnp.concatenate(nn, axis=1)
            out_v[pl.ds(row0 + g * 8, 8), :] = jnp.concatenate(ov, axis=1).astype(bf16)
            ends.append(orall([pltpu.bitcast(o, u32) for o in ov[PT:]]))
            fin(dl, ends[-1])

        def p4(g, n, dl):
            rg = (p3s.pop(g) + mrow(9, 0)).astype(bf16).astype(f32)
            m = g % 4
            if n % GM == 0:
                bst['v'] = best_v[m * 8:(m + 1) * 8, :]
                bst['i'] = besti_v[m * 8:(m + 1) * 8, :]
            upd = rg > bst['v']
            bst['v'] = jnp.where(upd, rg, bst['v'])
            bst['i'] = jnp.where(upd, row0 + g * 8, bst['i'])
            if n % GM == GM - 1:
                best_v[m * 8:(m + 1) * 8, :] = bst['v']
                besti_v[m * 8:(m + 1) * 8, :] = bst['i']
            if n % 2 == 1:
                fin(dl, pltpu.bitcast(bst['i'], u32))

        def emit(i, tk):
            if i < NG:
                p1(order[i], tk())
            if 0 <= i - 1 < NG:
                p3(order[i - 1], slots[i - 1] + WP)
            if 0 <= i - 2 < NG:
                p4(order[i - 2], i - 2, slots[i - 2] + WP + 2)
            if snap is not None and i - 2 == SNAP * GM - 1:
                snap()
            if i == NG:
                end()
                if snap is not None:
                    spec.append(orall(ends[SNAP * GM:]))
        return slots + [slots[-1] + 1, slots[-1] + 2], emit

    def st_perm(t, js, slots, fin, dl, r0=0):
        cst = {}

        def emit(i_, tk):
            r = r0 + i_
            if i_ == 0:
                lane = lax.broadcasted_iota(i32, (8, 128), 1)
                cls = (lane // 4) % 5
                cst['m'] = [cls == c for c in range(1, NJ)]
                for j in js:
                    cst[j] = 4 * ((5 * (lane % 32) + j) % 32) + lane // 32
            srcs = [tou(wqkv_raw[r * 16:(r + 1) * 16, t * D + i * 128:t * D + (i + 1) * 128]) for i in range(NJ)]
            for j in js:
                m = srcs[(j * 3) % 5]
                if tk() is not None:
                    m = m | tk()
                for c in range(1, NJ):
                    m = jnp.where(cst['m'][c - 1], srcs[((j + 5 - c) * 3) % 5], m)
                m = jnp.take_along_axis(m, cst[j], axis=1)
                wq_p[t * NJ + j][r * 8:(r + 1) * 8, :] = m
            if fin is not None:
                fin(slots[i_] + dl, m)
        return slots, emit

    def st_perm_o(slots, fin, dl):
        def emit(i, tk):
            n, j = (i % 25) // NJ, i % NJ
            if i < 25:
                w = wo_raw[j * 128:(j + 1) * 128, n * 128:(n + 1) * 128].astype(f32) * (
                    mrow(2, n) + pltpu.bitcast(tk(), f32))[0:1]
                wo_f[n, j * 128:(j + 1) * 128, :] = w
                fin(slots[i] + dl, pltpu.bitcast(w[120:128], u32))
                return
            for dd in range(4):
                for hh in range(2):
                    r0 = hh * 16 * DH + 4 * j + dd
                    ev = wo_f[n, pl.ds(r0, 8, stride=2 * DH), :]
                    od = wo_f[n, pl.ds(r0 + DH, 8, stride=2 * DH), :]
                    p0 = j * 64 + dd * 16 + hh * 8
                    pk = pack2(ev, od)
                    wo_p[n][p0:p0 + 8, :] = pk
            fin(slots[i] + dl, pk)
        return slots, emit

    class Phase:
        def __init__(self, carry=None):
            self.done = {}
            self.tok = None
            if carry is not None:
                self.done = dict(carry.left)
                self.tok = carry.tok
            self.cur = 0

        def fin(self, slot, v):
            self.done.setdefault(max(slot, self.cur), []).append(v)

        def run(self, jobs, streams):
            pos = [0] * len(streams)
            pend = []
            for c in range(len(jobs) + 1):
                self.cur = c
                cache = []

                def tk():
                    if self.tok is None:
                        return None
                    if not cache:
                        cache.append(zand(self.tok))
                    return cache[0]
                for si, (slots, emit) in enumerate(streams):
                    while pos[si] < len(slots) and (slots[pos[si]] <= c or c == len(jobs)):
                        emit(pos[si], tk)
                        pos[si] += 1
                if c == len(jobs):
                    break
                pend += self.done.pop(c, [])
                r = jobs[c](pend)
                if r is not None:
                    self.tok = r
                    pend = []
            self.left = {k - len(jobs): v for k, v in self.done.items()}

    def out_cp(t):
        return pltpu.make_async_copy(out_v.at[pl.ds(t * TM, TM)], out_hbm.at[pl.ds(t * TM, TM)], sems.at[1])

    best_v[...] = jnp.full((32, 128), -jnp.inf, f32)
    besti_v[...] = jnp.zeros((32, 128), i32)
    for r_ in (ka, kb, kc, va, vb, vc):
        for j in range(NJ):
            r_[j, KVR - 8:KVR, :] = jnp.zeros((8, 128), f32)
    wait(g_z)
    zv = pltpu.bitcast(zero_v[...], i32)
    for i in range(4):
        zs[i] = zv[i, 0]
    wait(g_x0)
    cf = c_v[...].astype(f32)
    sc_v[...] = tou(jnp.broadcast_to((cf * jax.nn.sigmoid(cf)).astype(bf16), (16, D)))
    for g in range(NG):
        xf = [x_v[g * 8:(g + 1) * 8, j * 128:(j + 1) * 128].astype(f32) for j in range(NJ)]
        m_, rs_ = stats(lsum(tree(xf)), lsum(tree([x * x for x in xf])))
        h2_v[g * 8:(g + 1) * 8, :] = jnp.concatenate([(x - m_) * rs_ for x in xf], axis=1)
    wait(g_ca)
    for j in range(NJ):
        job_mod(1, j)([])
    Phase().run([], [st_apply(0, [0] * 16, None)])
    wait(g_wq)

    ph = Phase()
    fin = ph.fin
    mo = [2, 3, 0, 1]
    nat = list(range(NM))
    jobs, streams, spec = [], [], []

    def nmaj(t, ns, bias=False):
        return [job_qkv(t, n, m, (1 if m == 0 else 2) if bias == 1 else bias) for n in ns for m in nat]

    def mmaj(t, ns):
        return [job_qkv(t, n, m) for m in mo for n in ns]

    def waiter(g, *keys):
        def f():
            wait(g)
        return job_call(f)

    QS, KS, VS = range(NJ), range(NJ, 2 * NJ), range(2 * NJ, 3 * NJ)
    K3 = 52; K5 = 6; K4 = 2
    K1 = 18
    KX = 20; PH = 1; PL = 0; L0 = 36
    jobs += [job_q0(n, m, hi) for hi in range(2) for n in QS for m in nat]
    jobs += mmaj(1, QS) + nmaj(0, KS) + nmaj(1, KS)[:KX]
    jobs.insert(80 + KX - K5, waiter(g_wv, ('raw', 2), 'x2'))
    for j in range(NJ):
        jobs.insert(80 + KX - K5 + 1 + [j, 2 * j, (3 * j) // 2, 2 * j + 1][1], job_mod(0, j))
    jobs.insert(K1, waiter(g_wq2, 'x1'))
    jobs.insert(K3, waiter(g_wk, ('raw', 1)))
    s5 = 83 + KX - K5
    sv0 = len(jobs)
    for j in range(NJ):
        jobs += nmaj(0, [2 * NJ + j], 1) + [job_bq(j)]
    sk1 = len(jobs)
    jobs += nmaj(1, KS)[KX:]
    sv1 = len(jobs)
    for j in range(NJ):
        jobs += nmaj(1, [2 * NJ + j], 2) + [job_bq(NJ + j)]
    jobs.insert(len(jobs) - K4, waiter(g_xr, 'x'))
    s4 = len(jobs) - K4
    for j in range(NJ):
        streams.append(st_perm(0, [j], [[0, 0, PL, 1, 3][j]] * QLO, None, 0))
        streams.append(st_perm(0, [j], [K1 + [1, 1, 1, 1 + PH, 1 + 3 * PH][j]] * (40 - QLO), None, 0, QLO))
    streams.append(st_ln1(1, _spread(12, K1 + 1, L0) + _spread(NG - 12, L0, 48), fin, mo))
    PK = 4; PV = 10
    streams += [st_perm(1, [j], _spread(40, K3 + 1 + PK * j, K3 + 1 + PK * (j + 1)), None, 0) for j in range(NJ)]
    streams += [st_perm(2, [j], _spread(40, max(s5, sv0 + 5 * j - PV), max(s5 + 1, sv0 + 5 * j - PV + 5)), None, 0)
                for j in range(NJ)]
    st = {}
    for t in range(2, NT):
        if t == 6:
            jobs.append(waiter(g_rest))
        st[t] = len(jobs)
        jl = mmaj(t, QS) + nmaj(t, KS) + nmaj(t, VS) if t < NT - 1 else mmaj(t, KS) + nmaj(t, VS) + mmaj(t, QS)
        for i, jb in enumerate(jl):
            jobs.append(jb)
            if t == 6 and i % 3 == 1:
                jobs.append(job_mod(2 + (i // 3) // NJ, (i // 3) % NJ))

    def consts():
        cb, sb, gbv = mod_v[:, 4 * D:5 * D], mod_v[:, 3 * D:4 * D], mod_v[:, 5 * D:6 * D]
        wr = jnp.broadcast_to(wr_v[...].astype(f32).reshape(1, D), (8, D))
        mod_v[:, 6 * D:7 * D] = gbv * cb
        mod_v[:, 7 * D:8 * D] = gbv * sb
        mod_v[:, 8 * D:9 * D] = cb * wr
        mod_v[:, 9 * D:9 * D + 128] = jnp.broadcast_to(lsum(sb * wr), (8, 128))

    jobs.insert(st[7] + 20, job_call(consts))
    f6, f7 = st[7], len(jobs)

    def argmax(row):
        bv = best_v[...]
        bi = besti_v[...] + (lax.broadcasted_iota(i32, (32, 128), 0) & 7)
        mx = jnp.max(bv, axis=0, keepdims=True)
        cand = jnp.where(bv == mx, bi, S)
        idxv = jnp.min(cand, axis=0, keepdims=True)
        idx = jnp.minimum(idxv, S - 1)[0, 0]
        return mx, idx, h2_v[pl.ds(idx, 1), :] if row else None

    def gap(n, lo, hi, bar, taper):
        return [x if x < bar - taper else x + taper + 1 for x in _spread(n, lo, hi - taper - 1)]

    TP = 5; AX = 22; AY = 4; LX = -10
    streams += [st_halo(0, 2, _spread(NJ, sv0 + 4, sv0 + 20)), st_halo(0, 3, _spread(NJ, sk1 + 4, sk1 + 14)),
                st_halo(1, 2, _spread(NJ, sv1 + 4, sv1 + 14)), st_halo(1, 3, _spread(NJ, st[2] + 4, st[2] + 16))]
    for t in range(2, NT - 1):
        streams += [st_halo(t, 2, _spread(NJ, st[t + 1] - 16, st[t + 1] - 6)),
                    st_halo(t, 3, _spread(NJ, st[t + 1] + 4, st[t + 1] + 16))]
    streams += [st_halo(7, 2, _spread(NJ, f6 + 28, f6 + 42)), st_halo(7, 3, _spread(NJ, f6 + 48, f6 + 60))]
    a_lo = [sk1 + 2, st[2] + AX, st[3] + AX - AY, st[4] + AX - 2 * AY, st[5] + max(AX - 3 * AY, 1)]
    streams.append(st_attention(0, gap(NG, a_lo[0], a_lo[1], s4 - 1, TP), fin))
    for t in range(1, 4):
        streams.append(st_attention(t, _spread(NG, a_lo[t], a_lo[t + 1]), fin))
    A5 = 4
    streams.append(st_attention(4, gap(NG, a_lo[4], st[6] + A5, st[6] - 1, ATHI - 1), fin))
    T0 = 0; T1 = 46; T2 = 48; T3 = 136; T4 = 10; T5 = 8
    streams.append(st_attention(5, _spread(NG, st[6] + A5, f6 + T0), fin))
    streams.append(st_attention(6, _spread(NG, f6 + max(T0, 1), f6 + T1), fin))
    streams.append(st_attention(7, _spread(T4, f6 + T2, f7 + T5) + _spread(NG - T4, f7 + T5, f7 + T3), fin,
                                order=[(i + 16) % NG for i in range(NG)]))
    streams.append(st_ln1(2, _spread(NG, s5 + 10, sk1 + 4), fin, mo))
    for t in range(3, 6):
        streams.append(st_ln1(t, _spread(NG, max(st[t - 1] + LX, s4), st[t] + LX), fin, mo))
    streams.append(st_ln1(6, _spread(NG, st[5] + LX, st[6] - LNHI), fin, mo))
    streams.append(st_ln1(7, _spread(NG, st[6], st[7] + 0), fin, mo))
    streams.append(st_perm_o(_spread(25, f6 + 4, f6 + 24) + _spread(25, f6 + 26, f6 + 54), fin, 4))
    for t in range(NT):
        mt = mo if t == NT - 1 else nat
        jobs += [job_wo(t, c, m) for m in mt for c in range(NJ)]
        s0 = f7 + 20 * t + POLO
        sl = _spread(NG, s0, s0 + 20)
        if t == NT - 1:
            sl = [min(sl[i], s0 - POLO + PL7 + 5 * (i // 8) + (i % 8) // 3) for i in range(NG)]
        streams.append(st_post(t, sl, fin, mt, out_cp(t).start,
                               (lambda: spec.append(argmax(True))) if t == NT - 1 else None))
    ph.run(jobs, streams)

    def moe(mx, idx, nrow, after=None):
        base = pl.multiple_of((idx // 16) * 16, 16)
        hrow = jnp.broadcast_to(nrow, (8, D)) * mod_v[:, 4 * D:5 * D] + mod_v[:, 3 * D:4 * D]
        hrow = hrow.astype(bf16).astype(f32)
        hf = [hrow[:, j * 128:(j + 1) * 128] for j in range(NJ)]
        h16 = [tob(pack2(h, h)) for h in hf]
        NC = 7
        NV = (F - NC * 128) // 8

        def glu(g, u):
            hg = 0.5 * g
            return (hg * jnp.tanh(hg) + hg) * u

        def ntdot(w_v, c):
            return tree([lax.dot_general(h16[j], w_v[c * 128:(c + 1) * 128, j * 128:(j + 1) * 128],
                                         (((1,), (1,)), ((), ())),
                                         preferred_element_type=f32)[0:8] for j in range(NJ)])

        def wrow(w_v, r0, j):
            return w_v[r0:r0 + 8, j * 128:(j + 1) * 128].astype(f32)

        ym, acts, acc, toks = None, [], None, []
        MD = 2
        MA = 3
        NP = 2 * NC - 1 + MD
        for c in range(2 * NC + 2):
            if c < 2 * NC:
                toks.append(ntdot(wu_v if c % 2 else wg_v, c // 2))
                if c % 2:
                    a8 = glu(toks[c - 1], toks[c])
                    acts.append(tob(pack2(a8, a8)))
            if c > 2 and c % 2:
                k = (c - 3) // 2
                yc = [jnp.dot(acts[k], wd_v[k * 128:(k + 1) * 128, j * 128:(j + 1) * 128],
                              preferred_element_type=f32)[0:8] for j in range(NJ)]
                ym = yc if ym is None else [ym[j] + yc[j] for j in range(NJ)]
            if c < NP:
                tk_ = None if c < MD else pltpu.bitcast(toks[c - MD], u32)
                if after is not None and c == MA:
                    tk_ = after if tk_ is None else tk_ | after
                h0 = hf if tk_ is None else [h + pltpu.bitcast(zand(tk_), f32) for h in hf]
                for i in range(c * NV // NP, (c + 1) * NV // NP):
                    r0 = NC * 128 + i * 8
                    g = lsum(tree([wrow(wg_v, r0, j) * h0[j] for j in range(NJ)]))
                    u = lsum(tree([wrow(wu_v, r0, j) * h0[j] for j in range(NJ)]))
                    av = glu(g, u)
                    pr = [wrow(wd_v, r0, j) * av for j in range(NJ)]
                    acc = pr if acc is None else [acc[j] + pr[j] for j in range(NJ)]
        y = jnp.concatenate(ym, axis=1)[0:1] + jnp.sum(jnp.concatenate(acc, axis=1), axis=0, keepdims=True)
        y = y * jax.nn.sigmoid(mx[:, 0:1])
        rows = base + lax.broadcasted_iota(i32, (16, D), 0)
        gb = mod_v[0:1, 5 * D:6 * D]
        old = out_v[pl.ds(base, 16), :].astype(f32)
        newblk = jnp.where(rows == idx, old + gb * y, old)
        fix_v[...] = newblk.astype(bf16)

    moe(*spec[0], spec[1])
    mx_f, idx_f, _ = argmax(False)
    for t in range(NT):
        out_cp(t).wait()

    @pl.when(idx_f != spec[0][1])
    def _():
        moe(mx_f, idx_f, h2_v[pl.ds(idx_f, 1), :])

    base_f = pl.multiple_of((idx_f // 16) * 16, 16)
    fix = pltpu.make_async_copy(fix_v, out_hbm.at[pl.ds(base_f, 16)], sems.at[0])
    fix.start()
    fix.wait()


@jax.jit
def pallas_adaLN_cond__sliding_local_dilated__moe_arch_mod__prompt_kernel(
    A_x, A_wqkv, A_wo, B_x, B_w_r, B_w_gate, B_w_up, B_w_down, c, w_mod,
):
    x = A_x.reshape(S, D)
    V = pltpu.VMEM
    scratch = [V((D // 2, 128), u32)] * 20 + [V((NJ, MS, 128), f32)] * 8 + [
        V((1, S, D), bf16),
        V((3 * NJ + 1, 8, 128), f32),
        V((D, 3 * D), bf16),
        V((D, D), bf16),
        V((NJ, D, 128), f32),
        V((F, D), bf16),
        V((F, D), bf16),
        V((F, D), bf16),
        V((D, 6 * D), bf16),
        V((8, 9 * D + 128), f32),
        V((NJ, TM // 2, 128), u32), V((NJ, TM // 2, 128), u32), V((NJ, TM // 2, 128), u32),
        V((NJ, TM, 128), f32), V((NJ, TM, 128), f32), V((NJ, TM, 128), f32),
        V((NJ, KVR, 128), f32), V((NJ, KVR, 128), f32), V((NJ, KVR, 128), f32),
        V((NJ, KVR, 128), f32), V((NJ, KVR, 128), f32), V((NJ, KVR, 128), f32),
        V((NT - 1, NJ, TM // 2, 128), u32), V((NJ, TM // 2, 128), u32),
        V((S, D), f32),
        V((S, D), bf16),
        V((32, 128), f32),
        V((32, 128), i32),
        V((8, 128), u32),
        V((8, 128), u32),
        V((8, D), u32),
        V((8, D), u32),
        V((16, D), bf16),
        V((1, D), bf16),
        V((D,), bf16),
        pltpu.SMEM((4,), i32),
        pltpu.SemaphoreType.DMA((NSEM,)),
    ]
    out = pl.pallas_call(
        _kernel,
        out_shape=jax.ShapeDtypeStruct((S, D), bf16),
        in_specs=[pl.BlockSpec(memory_space=pltpu.HBM)] * 9,
        out_specs=pl.BlockSpec(memory_space=pltpu.HBM),
        scratch_shapes=scratch,
        compiler_params=pltpu.CompilerParams(vmem_limit_bytes=100 * 2**20),
    )(x, A_wqkv, A_wo, B_w_r, B_w_gate.T, B_w_up.T, B_w_down, c, w_mod)
    return out.reshape(1, S, D)
```

```python
import math

import jax
import jax.numpy as jnp
from jax import lax
import jax.experimental.pallas as pl
import jax.experimental.pallas.tpu as pltpu


S = 2048
D = 640
H = 32
DH = 20
WIN = 8
F = 1728
NJ = D // 128
TM = 256
NT = S // TM
NG = TM // 8
HV = 14
MS = 64
NM = TM // MS
GM = MS // 8
KVR = (HV + NG + 1) * 8
EPS = 1e-5
LOG2E = math.log2(math.e)
QSCALE = (DH ** -0.5) * LOG2E
NEG = -1000000000.0 * LOG2E
f32 = jnp.float32
bf16 = jnp.bfloat16
u32 = jnp.uint32
i32 = jnp.int32
KL = 3
QLO = 8 * KL
NSEM = 12

WA = 20
WL = 16
WP = 11
CH = 2
ATHI = 8
LNHI = 4
POLO = 6
PL7 = 6
PT = 2
SNAP = 4
ST = 4
NE = 168
NC = 3
WM = 12
WA2 = 16
WA3 = 16
FA = 5
FL = 5


def _spread(n, lo, hi):
    return [int(lo + (i * (hi - lo)) / n) for i in range(n)]


def _kernel(x_hbm, wqkv_hbm, wo_hbm, wr_hbm, wg_hbm, wu_hbm, wd_hbm, c_hbm, wmod_hbm,
            out_hbm, *wp):
    (x_3, bias_v, wqkv_raw, wo_raw, wo_f, wg_v, wu_v, wd_v, wmod_v,
     mod_v, ha, hb, hc, qa, qb, qc, ka, kb, kc, va, vb, vc, o_all, oc, h2_v, out_v, best_v, besti_v,
     zsrc, zero_v, sc_v, sap_v, fix_v, c_v, wr_v, zs, sems) = wp[28:]
    x_v = x_3.at[0]
    wq_p = wp[:15]
    wo_p = wp[15:20]
    x1s = wp[20:28]

    def cp(src, dst, i):
        n = src.shape[0]
        if n < 64 or not 0:
            return [(pltpu.make_async_copy(src, dst, sems.at[i]), 0)]
        return [(pltpu.make_async_copy(src.at[pl.ds(p * n // 2, n // 2)], dst.at[pl.ds(p * n // 2, n // 2)],
                                       sems.at[i]), p * 0) for p in range(2)]

    def xcp(t0, nt, i):
        return cp(x_hbm.at[pl.ds(t0 * TM, nt * TM)], x_v.at[pl.ds(t0 * TM, nt * TM)], i)

    def colcp(src, dst, k0, nk, i, r0=0, nr=D):
        return cp(src.at[pl.ds(r0, nr), pl.ds(k0 * D, nk * D)], dst.at[pl.ds(r0, nr), pl.ds(k0 * D, nk * D)], i)

    def wait(g):
        for d, _ in g:
            d.wait()

    g_z = cp(zsrc, zero_v, 0)
    g_x0 = xcp(0, 1, 1) + cp(c_hbm, c_v, 1)
    g_wq = colcp(wqkv_hbm, wqkv_raw, 0, 1, 2, 0, 16 * QLO)
    g_wq2 = colcp(wqkv_hbm, wqkv_raw, 0, 1, 10, 16 * QLO, D - 16 * QLO) + xcp(1, 1, 10)
    g_ca = colcp(wmod_hbm, wmod_v, 1, 1, 3)
    g_wk = colcp(wqkv_hbm, wqkv_raw, 1, 1, 4)
    g_wv = colcp(wqkv_hbm, wqkv_raw, 2, 1, 5) + colcp(wmod_hbm, wmod_v, 0, 1, 5) + xcp(2, 1, 5)
    g_xr = xcp(3, 5, 6)
    g_rest = (colcp(wmod_hbm, wmod_v, 2, 4, 7) + cp(wo_hbm, wo_raw, 11) + [(pltpu.make_async_copy(wr_hbm, wr_v, sems.at[11]), 0)]
              + cp(wg_hbm, wg_v, 8) + cp(wu_hbm, wu_v, 9) + cp(wd_hbm, wd_v, 11))
    zsrc[...] = jnp.zeros((8, 128), u32)
    for d, p in g_x0 + g_ca + g_wq + g_wq2 + g_z + g_wk + g_wv + g_xr + g_rest:
        d.start(priority=p)

    BUF = [(ha, qa, ka, va), (hb, qb, kb, vb), (hc, qc, kc, vc)]

    def tob(u):
        return pltpu.bitcast(u, bf16)

    def tou(b):
        return pltpu.bitcast(b, u32)

    def pack2(a, b):
        return pltpu.bitcast(pltpu.pack_elementwise([a, b], packed_dtype=bf16), u32)

    def zand(v):
        return pltpu.bitcast(v, u32) & zero_v[...]

    def orall(vs):
        r = vs[0]
        for v in vs[1:]:
            r = r | v
        return r

    def mrow(k, j):
        return mod_v[:, k * D + j * 128:k * D + (j + 1) * 128]

    def tree(vs):
        return ((vs[0] + vs[1]) + (vs[2] + vs[3])) + vs[4]

    def lsum(v):
        return jnp.sum(v, axis=-1, keepdims=True)

    def stats(s, s2):
        m = s * (1.0 / D)
        v = jnp.maximum(s2 * (1.0 / D) - m * m, 0.0)
        return m, jnp.exp2(jnp.log(v + EPS) * (-0.5 * LOG2E))

    def zo(i):
        return pl.multiple_of(zs[i], 8)

    def oref(t):
        return oc if t == NT - 1 else o_all.at[t]

    def gated(w, toks):
        if toks:
            t = orall(toks) & zero_v[...]
            w = jnp.concatenate([w[0:8] | t, w[8:]], axis=0)
        return tob(w)

    def lhs(ref, m, extra=None):
        a = jnp.concatenate([ref[j, m * MS // 2:(m + 1) * MS // 2] for j in range(NJ)], axis=1)
        if extra is not None:
            a = jnp.concatenate([a, extra], axis=0)
        return tob(a)

    def job_qkv(t, n, m, bias=0):
        h_r, q_r, k_r, v_r = BUF[t % 3]

        def run(toks):
            res = jnp.dot(lhs(h_r, m, sap_v[...] if bias == 1 else None),
                          gated(wq_p[n][pl.ds(zo(m), D // 2), :], toks),
                          preferred_element_type=f32)
            if bias:
                if bias == 1:
                    bb = res[MS:MS + 8]
                    bias_v[n] = bb
                else:
                    bb = bias_v[n, pl.ds(zo(m), 8), :]
                res = jnp.concatenate([res[i * 8:(i + 1) * 8] + bb for i in range(GM)], axis=0)
            if n < NJ:
                q_r[n, m * MS:(m + 1) * MS, :] = res
            elif n < 2 * NJ:
                k_r[n - NJ, HV * 8 + m * MS:HV * 8 + (m + 1) * MS, :] = res
            else:
                v_r[n - 2 * NJ, HV * 8 + m * MS:HV * 8 + (m + 1) * MS, :] = res
            return res[0:8]
        return run

    def job_q0(n, m, hi):
        js = range(KL, NJ) if hi else range(KL)

        def run(toks):
            a = jnp.concatenate([ha[j, m * MS // 2:(m + 1) * MS // 2] for j in js], axis=1)
            res = jnp.dot(tob(a), gated(wq_p[n][pl.ds(js[0] * 64 + zo(m), len(js) * 64), :], toks),
                          preferred_element_type=f32)
            if hi:
                res = res + qa[n, m * MS:(m + 1) * MS, :]
            qa[n, m * MS:(m + 1) * MS, :] = res
            return res[0:8]
        return run

    def job_bq(n):
        def run(toks):
            bias_v[n] = jnp.dot(tob(sap_v[...]), tob(wq_p[n][pl.ds(zo(0), D // 2), :]),
                                preferred_element_type=f32)[0:8]
            return None
        return run

    def job_wo(t, c, m):
        o_r, x1_r, row0 = oref(t), x1s[4 * (t % 2) + m], t * TM

        def run(toks):
            a = jnp.dot(lhs(o_r, m), gated(wo_p[c][pl.ds(zo(m), D // 2), :], toks),
                        preferred_element_type=f32)
            for ci in range(GM):
                cc = m * GM + ci
                g = 4 * (cc % 8) + cc // 8
                xr = x_v[pl.ds(row0 + g * 8, 8), c * 128:(c + 1) * 128].astype(f32)
                x1_r[c, ci * 8:(ci + 1) * 8, :] = xr + a[ci * 8:(ci + 1) * 8]
            return a[0:8]
        return run

    def job_mod(k, j):
        def run(toks):
            lo = k * D + j * 128
            m = jnp.dot(tob(sc_v[...]), wmod_v[:, lo:lo + 128], preferred_element_type=f32).astype(bf16)
            if k == 0:
                sap_v[:, j * 128:(j + 1) * 128] = tou(m)
            m = m[:8].astype(f32)
            if k in (1, 4):
                m = m + 1.0
            mod_v[:, lo:lo + 128] = m
            return None
        return run

    def job_call(fn):
        def run(toks):
            fn()
            return None
        return run

    def st_attention(t, slots, fin, order=None):
        _, q_c, k_c, v_c = BUF[t % 3]
        o_c = oref(t)
        first = t == 0
        st1, st2, outs, chain = {}, {}, {}, []
        order = order or [(i + HV) % NG for i in range(NG)]

        def ld(ref, j, i):
            return ref[j, (HV + i) * 8:(HV + i + 1) * 8, :]

        def a1(g, tok):
            if CH and len(chain) >= CH:
                ct = zand(chain[-CH])
                tok = ct if tok is None else tok | ct
            sc = QSCALE if tok is None else pltpu.bitcast(
                pltpu.bitcast(jnp.full((8, 128), QSCALE, f32), u32) | tok, f32)
            if t < 2:
                q = [(q_c[j, g * 8:(g + 1) * 8, :] + bias_v[j, pl.ds(zo(0), 8), :]) * sc for j in range(NJ)]
            else:
                q = [q_c[j, g * 8:(g + 1) * 8, :] * sc for j in range(NJ)]
            ps = []
            for w in range(WIN):
                p = q[0] * ld(k_c, 0, g - 2 * w)
                for j in range(1, NJ):
                    p = p + q[j] * ld(k_c, j, g - 2 * w)
                ps.append((p, pltpu.roll(p, 64, 1)))
            st1[g] = ps

        def a2(g):
            ps = []
            for (p, pr) in st1.pop(g):
                p = p + pr
                ps.append((p, pltpu.roll(p, 32, 1)))
            st2[g] = ps

        def a3(g, dl):
            ls = [p + pr for (p, pr) in st2.pop(g)]
            if first:
                sub = lax.broadcasted_iota(i32, (8, 128), 0)
                ls = [jnp.where(sub > 0, ls[w], NEG) if g - 2 * w < 0 else ls[w] for w in range(WIN)]
            m = jnp.maximum(jnp.maximum(jnp.maximum(ls[0], ls[1]), jnp.maximum(ls[2], ls[3])),
                            jnp.maximum(jnp.maximum(ls[4], ls[5]), jnp.maximum(ls[6], ls[7])))
            es = [jnp.exp2(l - m) for l in ls]
            den = ((es[0] + es[1]) + (es[2] + es[3])) + ((es[4] + es[5]) + (es[6] + es[7]))
            inv = pl.reciprocal(den, approx=True)
            o = []
            for j in range(NJ):
                acc = es[0] * ld(v_c, j, g)
                for w in range(1, WIN):
                    acc = acc + es[w] * ld(v_c, j, g - 2 * w)
                o.append(acc * inv)
            outs[g] = o
            chain.append(o[NJ - 1])
            if g % 2 == 1:
                o0 = outs.pop(g - 1)
                o1 = outs.pop(g)
                pk = [pack2(o0[j], o1[j]) for j in range(NJ)]
                for j in range(NJ):
                    o_c[j, pl.ds(32 * (g // 8) + (g // 2) % 4, 8, stride=4), :] = pk[j]
                if FA:
                    fin(dl, orall(pk[NJ - FA:]))

        def emit(i, tk):
            if i < NG:
                a1(order[i], tk())
            if 0 <= i - 1 < NG:
                a2(order[i - 1])
            if 0 <= i - 2 < NG:
                a3(order[i - 2], slots[i - 2] + (WA if t < 5 else WA2 if t < 7 else WA3))
        return slots + [slots[-1] + 1, slots[-1] + 2], emit

    def st_halo(t, kv, slots):
        dst, src = BUF[t % 3][kv], BUF[(t - 1) % 3][kv]

        def emit(j, tk):
            sub = lax.broadcasted_iota(i32, (8, 128), 0) | pltpu.bitcast(tk(), i32)
            for m in range(1, HV + 1):
                a0 = (HV + NG - m) * 8
                if t == 0:
                    top = 0.0
                else:
                    top = src[j, a0 + 7:a0 + 15, :]
                    if t == 2 and kv == 2:
                        top = top + bias_v[NJ + j]
                dst[j, (HV - m) * 8:(HV - m + 1) * 8, :] = jnp.where(sub < 1, top, dst[j, a0 - 1:a0 + 7, :])
        return slots, emit

    def st_ln1(t, slots, fin, mo):
        h_r, row0 = BUF[t % 3][0], t * TM
        l1, hs = {}, {}
        order = [2 * (4 * i + m) + p for m in mo for i in range(4) for p in range(2)]

        def ldx(g, z):
            r = 64 * (g // 8) + 8 * ((g // 2) % 4) + 32 * (g % 2)
            return [x_3[z, pl.ds(row0 + r, 8), j * 128:(j + 1) * 128].astype(f32) for j in range(NJ)]

        def n1(g, tok):
            xf = ldx(g, 0)
            xf[0] = xf[0] + pltpu.bitcast(tok, f32)
            l1[g] = (lsum(tree(xf)), lsum(tree([x * x for x in xf])))

        def n3(g, dl):
            m, rs = stats(*l1.pop(g))
            xf = ldx(g, zs[0])
            hs[g] = [(xf[j] - m) * rs * mrow(1, j) for j in range(NJ)]
            if t > 1:
                hs[g] = [hs[g][j] + mrow(0, j) for j in range(NJ)]
            if g % 2 == 1:
                b = g // 2
                h0 = hs.pop(g - 1)
                h1 = hs.pop(g)
                pk = [pack2(h0[j], h1[j]) for j in range(NJ)]
                for j in range(NJ):
                    h_r[j, pl.ds(32 * (b % 4) + b // 4, 8, stride=4), :] = pk[j]
                if FL:
                    fin(dl, orall(pk[NJ - FL:]))

        def emit(i, tk):
            if i < NG:
                n1(order[i], tk())
            if 0 <= i - 1 < NG:
                n3(order[i - 1], slots[i - 1] + (WL if t > 1 else 20 if i < 12 else 8))
        return slots + [slots[-1] + 1], emit

    def st_apply(t, slots, fin):
        order = sorted(range(NG // 2), key=lambda b: b % 4)

        def emit(i, tk):
            b = order[i]
            r = t * TM + 64 * (b // 4) + 8 * (b % 4)
            pk = [pack2(h2_v[r:r + 8, j * 128:(j + 1) * 128] * mrow(1, j),
                        h2_v[r + 32:r + 40, j * 128:(j + 1) * 128] * mrow(1, j)) for j in range(NJ)]
            for j in range(NJ):
                BUF[t][0][j, pl.ds(32 * (b % 4) + b // 4, 8, stride=4), :] = pk[j]
            if fin is not None:
                fin(slots[i] + 3, orall(pk))
        return slots, emit

    def st_post(t, slots, fin, mo, snap=None):
        x1_rs, row0 = x1s[4 * (t % 2):4 * (t % 2) + 4], t * TM
        p1s, p3s, bst, ends = {}, {}, {}, []
        order = [4 * ci + m for m in mo for ci in range(GM)]

        def ldx1(g, z):
            return [x1_rs[g % 4][j, pl.ds((g // 4) * 8 + zo(z), 8), :] for j in range(NJ)]

        def p1(g, tok):
            xf = ldx1(g, 0)
            if tok is not None:
                xf[0] = xf[0] + pltpu.bitcast(tok, f32)
            p1s[g] = (lsum(tree(xf)), lsum(tree([x * x for x in xf])))

        def p3(g, dl):
            x1 = ldx1(g, 1)
            m, rs = stats(*p1s.pop(g))
            nn = [(x1[j] - m) * rs for j in range(NJ)]
            ov = [(x1[j] + mrow(7, j)) + nn[j] * mrow(6, j) for j in range(NJ)]
            p3s[g] = lsum(tree([nn[j] * mrow(8, j) for j in range(NJ)]))
            h2_v[pl.ds(row0 + g * 8, 8), :] = jnp.concatenate(nn, axis=1)
            out_v[pl.ds(row0 + g * 8, 8), :] = jnp.concatenate(ov, axis=1).astype(bf16)
            ends.append(orall([pltpu.bitcast(o, u32) for o in ov[PT:]]))
            fin(dl, ends[-1])

        def p4(g, n, dl):
            rg = (p3s.pop(g) + mrow(9, 0)).astype(bf16).astype(f32)
            m = g % 4
            if n % GM == 0:
                bst['v'] = best_v[m * 8:(m + 1) * 8, :]
                bst['i'] = besti_v[m * 8:(m + 1) * 8, :]
            upd = rg > bst['v']
            bst['v'] = jnp.where(upd, rg, bst['v'])
            bst['i'] = jnp.where(upd, row0 + g * 8, bst['i'])
            if n % GM == GM - 1:
                best_v[m * 8:(m + 1) * 8, :] = bst['v']
                besti_v[m * 8:(m + 1) * 8, :] = bst['i']
            if n % 2 == 1:
                fin(dl, pltpu.bitcast(bst['i'], u32))

        def emit(i, tk):
            if i < NG:
                p1(order[i], tk())
            if 0 <= i - 1 < NG:
                p3(order[i - 1], slots[i - 1] + WP)
            if 0 <= i - 2 < NG:
                p4(order[i - 2], i - 2, slots[i - 2] + WP + 2)
            if snap is not None and i - 2 == SNAP * GM - 1:
                snap()
            if t == NT - 1 and i == 2 * GM:
                [cp_.start() for cp_ in last_cp(mo[0] // 2)]
            if i == NG:
                [cp_.start() for cp_ in (last_cp(mo[2] // 2) if t == NT - 1 else [out_cp(t)])]
                if t == NT - 1:
                    spec.append(orall(ends[2 * GM:]))
        return slots + [slots[-1] + 1, slots[-1] + 2], emit

    def st_perm(t, js, slots, fin, dl, r0=0):
        cst = {}

        def emit(i_, tk):
            r = r0 + i_
            if i_ == 0:
                lane = lax.broadcasted_iota(i32, (8, 128), 1)
                cls = (lane // 4) % 5
                cst['m'] = [cls == c for c in range(1, NJ)]
                for j in js:
                    cst[j] = 4 * ((5 * (lane % 32) + j) % 32) + lane // 32
            srcs = [tou(wqkv_raw[r * 16:(r + 1) * 16, t * D + i * 128:t * D + (i + 1) * 128]) for i in range(NJ)]
            for j in js:
                m = srcs[(j * 3) % 5]
                if tk() is not None:
                    m = m | tk()
                for c in range(1, NJ):
                    m = jnp.where(cst['m'][c - 1], srcs[((j + 5 - c) * 3) % 5], m)
                m = jnp.take_along_axis(m, cst[j], axis=1)
                wq_p[t * NJ + j][r * 8:(r + 1) * 8, :] = m
            if fin is not None:
                fin(slots[i_] + dl, m)
        return slots, emit

    def st_perm_o(slots, fin, dl):
        def emit(i, tk):
            n, j = (i % 25) // NJ, i % NJ
            if i < 25:
                w = wo_raw[j * 128:(j + 1) * 128, n * 128:(n + 1) * 128].astype(f32) * (
                    mrow(2, n) + pltpu.bitcast(tk(), f32))[0:1]
                wo_f[n, j * 128:(j + 1) * 128, :] = w
                fin(slots[i] + dl, pltpu.bitcast(w[120:128], u32))
                return
            for dd in range(4):
                for hh in range(2):
                    r0 = hh * 16 * DH + 4 * j + dd
                    ev = wo_f[n, pl.ds(r0, 8, stride=2 * DH), :]
                    od = wo_f[n, pl.ds(r0 + DH, 8, stride=2 * DH), :]
                    p0 = j * 64 + dd * 16 + hh * 8
                    pk = pack2(ev, od)
                    wo_p[n][p0:p0 + 8, :] = pk
            fin(slots[i] + dl, pk)
        return slots, emit

    class Phase:
        def __init__(self, carry=None):
            self.done = {}
            self.tok = None
            if carry is not None:
                self.done = dict(carry.left)
                self.tok = carry.tok
            self.cur = 0

        def fin(self, slot, v):
            self.done.setdefault(max(slot, self.cur), []).append(v)

        def run(self, jobs, streams):
            pos = [0] * len(streams)
            pend = []
            for c in range(len(jobs) + 1):
                self.cur = c
                cache = []

                def tk():
                    if self.tok is None:
                        return None
                    if not cache:
                        cache.append(zand(self.tok))
                    return cache[0]
                for si, (slots, emit) in enumerate(streams):
                    while pos[si] < len(slots) and (slots[pos[si]] <= c or c == len(jobs)):
                        emit(pos[si], tk)
                        pos[si] += 1
                if c == len(jobs):
                    break
                pend += self.done.pop(c, [])
                r = jobs[c](pend)
                if r is not None:
                    self.tok = r
                    pend = []
            self.left = {k - len(jobs): v for k, v in self.done.items()}

    def out_cp(t):
        return pltpu.make_async_copy(out_v.at[pl.ds(t * TM, TM)], out_hbm.at[pl.ds(t * TM, TM)],
                                     sems.at[1 if t <= ST else NSEM])

    def last_cp(h):
        rs = [(NT - 1) * TM + 32 * ci + 16 * h for ci in range(GM)]
        return [pltpu.make_async_copy(out_v.at[pl.ds(r, 16)], out_hbm.at[pl.ds(r, 16)], sems.at[NSEM]) for r in rs]

    def wait_late():
        for cp_ in [out_cp(t) for t in range(ST + 1, NT - 1)] + last_cp(0) + last_cp(1):
            cp_.wait()

    best_v[...] = jnp.full((32, 128), -jnp.inf, f32)
    besti_v[...] = jnp.zeros((32, 128), i32)
    for r_ in (ka, kb, kc, va, vb, vc):
        for j in range(NJ):
            r_[j, KVR - 8:KVR, :] = jnp.zeros((8, 128), f32)
    wait(g_z)
    zv = pltpu.bitcast(zero_v[...], i32)
    for i in range(4):
        zs[i] = zv[i, 0]
    wait(g_x0)
    cf = c_v[...].astype(f32)
    sc_v[...] = tou(jnp.broadcast_to((cf * jax.nn.sigmoid(cf)).astype(bf16), (16, D)))
    for g in range(NG):
        xf = [x_v[g * 8:(g + 1) * 8, j * 128:(j + 1) * 128].astype(f32) for j in range(NJ)]
        m_, rs_ = stats(lsum(tree(xf)), lsum(tree([x * x for x in xf])))
        h2_v[g * 8:(g + 1) * 8, :] = jnp.concatenate([(x - m_) * rs_ for x in xf], axis=1)
    wait(g_ca)
    for j in range(NJ):
        job_mod(1, j)([])
    Phase().run([], [st_apply(0, [0] * 16, None)])
    wait(g_wq)

    ph = Phase()
    fin = ph.fin
    mo = [2, 3, 0, 1]
    nat = list(range(NM))
    jobs, streams, spec = [], [], []

    def nmaj(t, ns, bias=False):
        return [job_qkv(t, n, m, (1 if m == 0 else 2) if bias == 1 else bias) for n in ns for m in nat]

    def mmaj(t, ns):
        return [job_qkv(t, n, m) for m in mo for n in ns]

    def waiter(g, *keys):
        def f():
            wait(g)
        return job_call(f)

    QS, KS, VS = range(NJ), range(NJ, 2 * NJ), range(2 * NJ, 3 * NJ)
    K3 = 52; K5 = 6; K4 = 2
    K1 = 18
    KX = 20; PH = 1; PL = 0; L0 = 36
    jobs += [job_q0(n, m, hi) for hi in range(2) for n in QS for m in nat]
    jobs += mmaj(1, QS) + nmaj(0, KS) + nmaj(1, KS)[:KX]
    jobs.insert(80 + KX - K5, waiter(g_wv, ('raw', 2), 'x2'))
    for j in range(NJ):
        jobs.insert(80 + KX - K5 + 1 + [j, 2 * j, (3 * j) // 2, 2 * j + 1][1], job_mod(0, j))
    jobs.insert(K1, waiter(g_wq2, 'x1'))
    jobs.insert(K3, waiter(g_wk, ('raw', 1)))
    s5 = 83 + KX - K5
    sv0 = len(jobs)
    for j in range(NJ):
        jobs += nmaj(0, [2 * NJ + j], 1) + [job_bq(j)]
    sk1 = len(jobs)
    jobs += nmaj(1, KS)[KX:]
    sv1 = len(jobs)
    for j in range(NJ):
        jobs += nmaj(1, [2 * NJ + j], 2) + [job_bq(NJ + j)]
    jobs.insert(len(jobs) - K4, waiter(g_xr, 'x'))
    s4 = len(jobs) - K4
    for j in range(NJ):
        streams.append(st_perm(0, [j], [[0, 0, PL, 1, 3][j]] * QLO, None, 0))
        streams.append(st_perm(0, [j], [K1 + [1, 1, 1, 1 + PH, 1 + 3 * PH][j]] * (40 - QLO), None, 0, QLO))
    streams.append(st_ln1(1, _spread(12, K1 + 1, L0) + _spread(NG - 12, L0, 48), fin, mo))
    PK = 4; PV = 10
    streams += [st_perm(1, [j], _spread(40, K3 + 1 + PK * j, K3 + 1 + PK * (j + 1)), None, 0) for j in range(NJ)]
    streams += [st_perm(2, [j], _spread(40, max(s5, sv0 + 5 * j - PV), max(s5 + 1, sv0 + 5 * j - PV + 5)), None, 0)
                for j in range(NJ)]
    st = {}
    for t in range(2, NT):
        if t == 6:
            jobs.append(waiter(g_rest))
        st[t] = len(jobs)
        jl = mmaj(t, QS) + nmaj(t, KS) + nmaj(t, VS) if t < NT - 1 else mmaj(t, KS) + nmaj(t, VS) + mmaj(t, QS)
        for i, jb in enumerate(jl):
            jobs.append(jb)
            if t == 6 and i % 3 == 1:
                jobs.append(job_mod(2 + (i // 3) // NJ, (i // 3) % NJ))

    def consts():
        cb, sb, gbv = mod_v[:, 4 * D:5 * D], mod_v[:, 3 * D:4 * D], mod_v[:, 5 * D:6 * D]
        wr = jnp.broadcast_to(wr_v[...].astype(f32).reshape(1, D), (8, D))
        mod_v[:, 6 * D:7 * D] = gbv * cb
        mod_v[:, 7 * D:8 * D] = gbv * sb
        mod_v[:, 8 * D:9 * D] = cb * wr
        mod_v[:, 9 * D:9 * D + 128] = jnp.broadcast_to(lsum(sb * wr), (8, 128))

    jobs.insert(st[7] + 20, job_call(consts))
    f6, f7 = st[7], len(jobs)

    def argmax(row):
        bv = best_v[...]
        bi = besti_v[...] + (lax.broadcasted_iota(i32, (32, 128), 0) & 7)
        mx = jnp.max(bv, axis=0, keepdims=True)
        cand = jnp.where(bv == mx, bi, S)
        idxv = jnp.min(cand, axis=0, keepdims=True)
        idx = jnp.minimum(idxv, ((ST + 1) * TM if row else S) - 1)[0, 0]
        return mx, idx, h2_v[pl.ds(idx, 1), :] if row else None

    def glu(g, u):
        hg = 0.5 * g
        return (hg * jnp.tanh(hg) + hg) * u

    def wrow(w_v, r0, j):
        return w_v[r0:r0 + 8, j * 128:(j + 1) * 128].astype(f32)

    def moe_in(nrow):
        hrow = jnp.broadcast_to(nrow, (8, D)) * mod_v[:, 4 * D:5 * D] + mod_v[:, 3 * D:4 * D]
        hrow = hrow.astype(bf16).astype(f32)
        return [hrow[:, j * 128:(j + 1) * 128] for j in range(NJ)]

    def vgroup(r0, h0, acc):
        g = lsum(tree([wrow(wg_v, r0, j) * h0[j] for j in range(NJ)]))
        u = lsum(tree([wrow(wu_v, r0, j) * h0[j] for j in range(NJ)]))
        av = glu(g, u)
        pr = [wrow(wd_v, r0, j) * av for j in range(NJ)]
        return pr if acc is None else [acc[j] + pr[j] for j in range(NJ)]

    early = {'acc': None}

    def st_moe(slots, fin):
        def emit(i, tk):
            if i == 0:
                early['hf'] = moe_in(spec[0][2])
            hf = early['hf']
            h0 = [hf[0] + pltpu.bitcast(tk(), f32)] + hf[1:]
            for k in (2 * i, 2 * i + 1):
                early['acc'] = vgroup(NC * 128 + k * 8, h0, early['acc'])
            fin(slots[i] + WM, orall([pltpu.bitcast(a, u32) for a in early['acc'][3:]]))
        return slots, emit

    def gap(n, lo, hi, bar, taper):
        return [x if x < bar - taper else x + taper + 1 for x in _spread(n, lo, hi - taper - 1)]

    TP = 5; AX = 22; AY = 4; LX = -10
    streams += [st_halo(0, 2, _spread(NJ, sv0 + 4, sv0 + 20)), st_halo(0, 3, _spread(NJ, sk1 + 4, sk1 + 14)),
                st_halo(1, 2, _spread(NJ, sv1 + 4, sv1 + 14)), st_halo(1, 3, _spread(NJ, st[2] + 4, st[2] + 16))]
    for t in range(2, NT - 1):
        streams += [st_halo(t, 2, _spread(NJ, st[t + 1] - 16, st[t + 1] - 6)),
                    st_halo(t, 3, _spread(NJ, st[t + 1] + 4, st[t + 1] + 16))]
    streams += [st_halo(7, 2, _spread(NJ, f6 + 28, f6 + 42)), st_halo(7, 3, _spread(NJ, f6 + 48, f6 + 60))]
    a_lo = [sk1 + 2, st[2] + AX, st[3] + AX - AY, st[4] + AX - 2 * AY, st[5] + max(AX - 3 * AY, 1)]
    streams.append(st_attention(0, gap(NG, a_lo[0], a_lo[1], s4 - 1, TP), fin))
    for t in range(1, 4):
        streams.append(st_attention(t, _spread(NG, a_lo[t], a_lo[t + 1]), fin))
    A5 = 4
    streams.append(st_attention(4, gap(NG, a_lo[4], st[6] + A5, st[6] - 1, ATHI - 1), fin))
    T0 = 0; T1 = 46; T2 = 48; T3 = 100; T4 = 10; T5 = 8
    streams.append(st_attention(5, _spread(NG, st[6] + A5, f6 + T0), fin))
    streams.append(st_attention(6, _spread(NG, f6 + max(T0, 1), f6 + T1), fin))
    streams.append(st_attention(7, _spread(T4, f6 + T2, f7 + T5) + _spread(NG - T4, f7 + T5, f7 + T3), fin,
                                order=[(i + 16) % NG for i in range(NG)]))
    streams.append(st_ln1(2, _spread(NG, s5 + 10, sk1 + 4), fin, mo))
    for t in range(3, 6):
        streams.append(st_ln1(t, _spread(NG, max(st[t - 1] + LX, s4), st[t] + LX), fin, mo))
    streams.append(st_ln1(6, _spread(NG, st[5] + LX, st[6] - LNHI), fin, mo))
    streams.append(st_ln1(7, _spread(NG, st[6], st[7] + 0), fin, mo))
    streams.append(st_perm_o(_spread(25, f6 + 4, f6 + 24) + _spread(25, f6 + 26, f6 + 54), fin, 4))
    for t in range(NT):
        mt = mo if t == NT - 1 else nat
        jobs += [job_wo(t, c, m) for m in mt for c in range(NJ)]
        s0 = f7 + 20 * t + POLO
        sl = _spread(NG, s0, s0 + 20)
        if t == NT - 1:
            sl = [min(sl[i], s0 - POLO + PL7 + 5 * (i // 8) + (i % 8) // 3) for i in range(NG)]
        streams.append(st_post(t, sl, fin, mt,
                               (lambda: spec.append(argmax(True))) if t == ST else None))
    m0 = f7 + 20 * ST + POLO + 5 * SNAP + 2
    streams.append(st_moe(_spread(NE // 2, m0, f7 + 160 + 0), fin))
    ph.run(jobs, streams)

    def moe(mx, idx, hf, NC, n0, acc, after=None):
        base = pl.multiple_of((idx // 16) * 16, 16)
        h16 = [tob(pack2(h, h)) for h in hf]
        NV = (F - NC * 128) // 8 - n0

        def ntdot(w_v, c):
            return tree([lax.dot_general(h16[j], w_v[c * 128:(c + 1) * 128, j * 128:(j + 1) * 128],
                                         (((1,), (1,)), ((), ())),
                                         preferred_element_type=f32)[0:8] for j in range(NJ)])

        ym, acts, toks = None, [], []
        MD = 2
        MA = 2
        NP = 2 * NC - 1 + MD
        for c in range(2 * NC + 2):
            if c < 2 * NC:
                toks.append(ntdot(wu_v if c % 2 else wg_v, c // 2))
                if c % 2:
                    a8 = glu(toks[c - 1], toks[c])
                    acts.append(tob(pack2(a8, a8)))
            if c > 2 and c % 2:
                k = (c - 3) // 2
                yc = [jnp.dot(acts[k], wd_v[k * 128:(k + 1) * 128, j * 128:(j + 1) * 128],
                              preferred_element_type=f32)[0:8] for j in range(NJ)]
                ym = yc if ym is None else [ym[j] + yc[j] for j in range(NJ)]
            if c < NP:
                tk_ = None if c < MD else pltpu.bitcast(toks[c - MD], u32)
                if after is not None and c == MA:
                    tk_ = after if tk_ is None else tk_ | after
                h0 = hf if tk_ is None else [h + pltpu.bitcast(zand(tk_), f32) for h in hf]
                for i in range(c * NV // NP, (c + 1) * NV // NP):
                    acc = vgroup(NC * 128 + (n0 + i) * 8, h0, acc)
        y = jnp.concatenate(ym, axis=1)[0:1] + jnp.sum(jnp.concatenate(acc, axis=1), axis=0, keepdims=True)
        y = y * jax.nn.sigmoid(mx[:, 0:1])
        rows = base + lax.broadcasted_iota(i32, (16, D), 0)
        gb = mod_v[0:1, 5 * D:6 * D]
        old = out_v[pl.ds(base, 16), :].astype(f32)
        newblk = jnp.where(rows == idx, old + gb * y, old)
        fix_v[...] = newblk.astype(bf16)

    moe(spec[0][0], spec[0][1], early['hf'], NC, NE, early['acc'], spec[1])
    mx_f, idx_f, _ = argmax(False)
    idx_s = spec[0][1]
    for t in range(ST + 1):
        out_cp(t).wait()

    def fix(idx):
        base = pl.multiple_of((idx // 16) * 16, 16)
        return pltpu.make_async_copy(fix_v, out_hbm.at[pl.ds(base, 16)], sems.at[0])

    @pl.when(idx_f == idx_s)
    def _():
        fix(idx_s).start()
        wait_late()
        fix(idx_s).wait()

    @pl.when(idx_f != idx_s)
    def _():
        moe(mx_f, idx_f, moe_in(h2_v[pl.ds(idx_f, 1), :]), 7, 0, None)
        wait_late()
        fix(idx_f).start()
        fix(idx_f).wait()


@jax.jit
def pallas_adaLN_cond__sliding_local_dilated__moe_arch_mod__prompt_kernel(
    A_x, A_wqkv, A_wo, B_x, B_w_r, B_w_gate, B_w_up, B_w_down, c, w_mod,
):
    x = A_x.reshape(S, D)
    V = pltpu.VMEM
    scratch = [V((D // 2, 128), u32)] * 20 + [V((NJ, MS, 128), f32)] * 8 + [
        V((1, S, D), bf16),
        V((3 * NJ + 1, 8, 128), f32),
        V((D, 3 * D), bf16),
        V((D, D), bf16),
        V((NJ, D, 128), f32),
        V((F, D), bf16),
        V((F, D), bf16),
        V((F, D), bf16),
        V((D, 6 * D), bf16),
        V((8, 9 * D + 128), f32),
        V((NJ, TM // 2, 128), u32), V((NJ, TM // 2, 128), u32), V((NJ, TM // 2, 128), u32),
        V((NJ, TM, 128), f32), V((NJ, TM, 128), f32), V((NJ, TM, 128), f32),
        V((NJ, KVR, 128), f32), V((NJ, KVR, 128), f32), V((NJ, KVR, 128), f32),
        V((NJ, KVR, 128), f32), V((NJ, KVR, 128), f32), V((NJ, KVR, 128), f32),
        V((NT - 1, NJ, TM // 2, 128), u32), V((NJ, TM // 2, 128), u32),
        V((S, D), f32),
        V((S, D), bf16),
        V((32, 128), f32),
        V((32, 128), i32),
        V((8, 128), u32),
        V((8, 128), u32),
        V((8, D), u32),
        V((8, D), u32),
        V((16, D), bf16),
        V((1, D), bf16),
        V((D,), bf16),
        pltpu.SMEM((4,), i32),
        pltpu.SemaphoreType.DMA((NSEM + 1,)),
    ]
    out = pl.pallas_call(
        _kernel,
        out_shape=jax.ShapeDtypeStruct((S, D), bf16),
        in_specs=[pl.BlockSpec(memory_space=pltpu.HBM)] * 9,
        out_specs=pl.BlockSpec(memory_space=pltpu.HBM),
        scratch_shapes=scratch,
        compiler_params=pltpu.CompilerParams(vmem_limit_bytes=100 * 2**20),
    )(x, A_wqkv, A_wo, B_w_r, B_w_gate.T, B_w_up.T, B_w_down, c, w_mod)
    return out.reshape(1, S, D)
```

```python
import math

import jax
import jax.numpy as jnp
from jax import lax
import jax.experimental.pallas as pl
import jax.experimental.pallas.tpu as pltpu


S = 2048
D = 640
H = 32
DH = 20
WIN = 8
F = 1728
NJ = D // 128
TM = 256
NT = S // TM
NG = TM // 8
HV = 14
MS = 64
NM = TM // MS
GM = MS // 8
KVR = (HV + NG + 1) * 8
EPS = 1e-5
LOG2E = math.log2(math.e)
QSCALE = (DH ** -0.5) * LOG2E
NEG = -1000000000.0 * LOG2E
f32 = jnp.float32
bf16 = jnp.bfloat16
u32 = jnp.uint32
i32 = jnp.int32
KL = 3
QLO = 8 * KL
NSEM = 12

WA = 20
WL = 16
WP = 11
CH = 2
ATHI = 8
LNHI = 4
POLO = 6
PL7 = 6
PT = 3
SNAP = 4
ST = 4
NE = 168
NC = 3
WM = 12
WA2 = 18
WA3 = 16
FA = 5
FL = 5


def _spread(n, lo, hi):
    return [int(lo + (i * (hi - lo)) / n) for i in range(n)]


def _kernel(x_hbm, wqkv_hbm, wo_hbm, wr_hbm, wg_hbm, wu_hbm, wd_hbm, c_hbm, wmod_hbm,
            out_hbm, *wp):
    (x_3, bias_v, wqkv_raw, wo_raw, wo_f, wg_v, wu_v, wd_v, wmod_v,
     mod_v, ha, hb, hc, qa, qb, qc, ka, kb, kc, va, vb, vc, o_all, oc, h2_v, out_v, best_v, besti_v,
     zsrc, zero_v, sc_v, sap_v, fix_v, c_v, wr_v, zs, sems) = wp[28:]
    x_v = x_3.at[0]
    wq_p = wp[:15]
    wo_p = wp[15:20]
    x1s = wp[20:28]

    def cp(src, dst, i):
        n = src.shape[0]
        if n < 64 or not 0:
            return [(pltpu.make_async_copy(src, dst, sems.at[i]), 0)]
        return [(pltpu.make_async_copy(src.at[pl.ds(p * n // 2, n // 2)], dst.at[pl.ds(p * n // 2, n // 2)],
                                       sems.at[i]), p * 0) for p in range(2)]

    def xcp(t0, nt, i):
        return cp(x_hbm.at[pl.ds(t0 * TM, nt * TM)], x_v.at[pl.ds(t0 * TM, nt * TM)], i)

    def colcp(src, dst, k0, nk, i, r0=0, nr=D):
        return cp(src.at[pl.ds(r0, nr), pl.ds(k0 * D, nk * D)], dst.at[pl.ds(r0, nr), pl.ds(k0 * D, nk * D)], i)

    def wait(g):
        for d, _ in g:
            d.wait()

    g_z = cp(zsrc, zero_v, 0)
    g_x0 = xcp(0, 1, 1) + cp(c_hbm, c_v, 1)
    g_wq = colcp(wqkv_hbm, wqkv_raw, 0, 1, 2, 0, 16 * QLO)
    g_wq2 = colcp(wqkv_hbm, wqkv_raw, 0, 1, 10, 16 * QLO, D - 16 * QLO) + xcp(1, 1, 10)
    g_ca = colcp(wmod_hbm, wmod_v, 1, 1, 3)
    g_wk = colcp(wqkv_hbm, wqkv_raw, 1, 1, 4)
    g_wv = colcp(wqkv_hbm, wqkv_raw, 2, 1, 5) + colcp(wmod_hbm, wmod_v, 0, 1, 5) + xcp(2, 1, 5)
    g_xr = xcp(3, 5, 6)
    g_rest = (colcp(wmod_hbm, wmod_v, 2, 4, 7) + cp(wo_hbm, wo_raw, 11) + [(pltpu.make_async_copy(wr_hbm, wr_v, sems.at[11]), 0)]
              + cp(wg_hbm, wg_v, 8) + cp(wu_hbm, wu_v, 9) + cp(wd_hbm, wd_v, 11))
    zsrc[...] = jnp.zeros((8, 128), u32)
    for d, p in g_x0 + g_ca + g_wq + g_wq2 + g_z + g_wk + g_wv + g_xr + g_rest:
        d.start(priority=p)

    BUF = [(ha, qa, ka, va), (hb, qb, kb, vb), (hc, qc, kc, vc)]

    def tob(u):
        return pltpu.bitcast(u, bf16)

    def tou(b):
        return pltpu.bitcast(b, u32)

    def pack2(a, b):
        return pltpu.bitcast(pltpu.pack_elementwise([a, b], packed_dtype=bf16), u32)

    def zand(v):
        return pltpu.bitcast(v, u32) & zero_v[...]

    def orall(vs):
        r = vs[0]
        for v in vs[1:]:
            r = r | v
        return r

    def mrow(k, j):
        return mod_v[:, k * D + j * 128:k * D + (j + 1) * 128]

    def tree(vs):
        return ((vs[0] + vs[1]) + (vs[2] + vs[3])) + vs[4]

    def lsum(v):
        return jnp.sum(v, axis=-1, keepdims=True)

    def stats(s, s2):
        m = s * (1.0 / D)
        v = jnp.maximum(s2 * (1.0 / D) - m * m, 0.0)
        return m, jnp.exp2(jnp.log(v + EPS) * (-0.5 * LOG2E))

    def zo(i):
        return pl.multiple_of(zs[i], 8)

    def oref(t):
        return oc if t == NT - 1 else o_all.at[t]

    def gated(w, toks):
        if toks:
            t = orall(toks) & zero_v[...]
            w = jnp.concatenate([w[0:8] | t, w[8:]], axis=0)
        return tob(w)

    def lhs(ref, m, extra=None):
        a = jnp.concatenate([ref[j, m * MS // 2:(m + 1) * MS // 2] for j in range(NJ)], axis=1)
        if extra is not None:
            a = jnp.concatenate([a, extra], axis=0)
        return tob(a)

    def job_qkv(t, n, m, bias=0):
        h_r, q_r, k_r, v_r = BUF[t % 3]

        def run(toks):
            res = jnp.dot(lhs(h_r, m, sap_v[...] if bias == 1 else None),
                          gated(wq_p[n][pl.ds(zo(m), D // 2), :], toks),
                          preferred_element_type=f32)
            if bias:
                if bias == 1:
                    bb = res[MS:MS + 8]
                    bias_v[n] = bb
                else:
                    bb = bias_v[n, pl.ds(zo(m), 8), :]
                res = jnp.concatenate([res[i * 8:(i + 1) * 8] + bb for i in range(GM)], axis=0)
            if n < NJ:
                q_r[n, m * MS:(m + 1) * MS, :] = res
            elif n < 2 * NJ:
                k_r[n - NJ, HV * 8 + m * MS:HV * 8 + (m + 1) * MS, :] = res
            else:
                v_r[n - 2 * NJ, HV * 8 + m * MS:HV * 8 + (m + 1) * MS, :] = res
            return res[0:8]
        return run

    def job_q0(n, m, hi):
        js = range(KL, NJ) if hi else range(KL)

        def run(toks):
            a = jnp.concatenate([ha[j, m * MS // 2:(m + 1) * MS // 2] for j in js], axis=1)
            res = jnp.dot(tob(a), gated(wq_p[n][pl.ds(js[0] * 64 + zo(m), len(js) * 64), :], toks),
                          preferred_element_type=f32)
            if hi:
                res = res + qa[n, m * MS:(m + 1) * MS, :]
            qa[n, m * MS:(m + 1) * MS, :] = res
            return res[0:8]
        return run

    def job_bq(n):
        def run(toks):
            bias_v[n] = jnp.dot(tob(sap_v[...]), tob(wq_p[n][pl.ds(zo(0), D // 2), :]),
                                preferred_element_type=f32)[0:8]
            return None
        return run

    def job_wo(t, c, m):
        o_r, x1_r, row0 = oref(t), x1s[4 * (t % 2) + m], t * TM

        def run(toks):
            a = jnp.dot(lhs(o_r, m), gated(wo_p[c][pl.ds(zo(m), D // 2), :], toks),
                        preferred_element_type=f32)
            for ci in range(GM):
                cc = m * GM + ci
                g = 4 * (cc % 8) + cc // 8
                xr = x_v[pl.ds(row0 + g * 8, 8), c * 128:(c + 1) * 128].astype(f32)
                x1_r[c, ci * 8:(ci + 1) * 8, :] = xr + a[ci * 8:(ci + 1) * 8]
            return a[0:8]
        return run

    def job_mod(k, j):
        def run(toks):
            lo = k * D + j * 128
            m = jnp.dot(tob(sc_v[...]), wmod_v[:, lo:lo + 128], preferred_element_type=f32).astype(bf16)
            if k == 0:
                sap_v[:, j * 128:(j + 1) * 128] = tou(m)
            m = m[:8].astype(f32)
            if k in (1, 4):
                m = m + 1.0
            mod_v[:, lo:lo + 128] = m
            return None
        return run

    def job_call(fn):
        def run(toks):
            fn()
            return None
        return run

    def st_attention(t, slots, fin, order=None):
        _, q_c, k_c, v_c = BUF[t % 3]
        o_c = oref(t)
        first = t == 0
        st1, st2, outs, chain = {}, {}, {}, []
        order = order or [(i + HV) % NG for i in range(NG)]

        def ld(ref, j, i):
            return ref[j, (HV + i) * 8:(HV + i + 1) * 8, :]

        def a1(g, tok):
            if CH and len(chain) >= CH:
                ct = zand(chain[-CH])
                tok = ct if tok is None else tok | ct
            sc = QSCALE if tok is None else pltpu.bitcast(
                pltpu.bitcast(jnp.full((8, 128), QSCALE, f32), u32) | tok, f32)
            if t < 2:
                q = [(q_c[j, g * 8:(g + 1) * 8, :] + bias_v[j, pl.ds(zo(0), 8), :]) * sc for j in range(NJ)]
            else:
                q = [q_c[j, g * 8:(g + 1) * 8, :] * sc for j in range(NJ)]
            ps = []
            for w in range(WIN):
                p = q[0] * ld(k_c, 0, g - 2 * w)
                for j in range(1, NJ):
                    p = p + q[j] * ld(k_c, j, g - 2 * w)
                ps.append((p, pltpu.roll(p, 64, 1)))
            st1[g] = ps

        def a2(g):
            ps = []
            for (p, pr) in st1.pop(g):
                p = p + pr
                ps.append((p, pltpu.roll(p, 32, 1)))
            st2[g] = ps

        def a3(g, dl):
            ls = [p + pr for (p, pr) in st2.pop(g)]
            if first:
                sub = lax.broadcasted_iota(i32, (8, 128), 0)
                ls = [jnp.where(sub > 0, ls[w], NEG) if g - 2 * w < 0 else ls[w] for w in range(WIN)]
            m = jnp.maximum(jnp.maximum(jnp.maximum(ls[0], ls[1]), jnp.maximum(ls[2], ls[3])),
                            jnp.maximum(jnp.maximum(ls[4], ls[5]), jnp.maximum(ls[6], ls[7])))
            es = [jnp.exp2(l - m) for l in ls]
            den = ((es[0] + es[1]) + (es[2] + es[3])) + ((es[4] + es[5]) + (es[6] + es[7]))
            inv = pl.reciprocal(den, approx=True)
            o = []
            for j in range(NJ):
                acc = es[0] * ld(v_c, j, g)
                for w in range(1, WIN):
                    acc = acc + es[w] * ld(v_c, j, g - 2 * w)
                o.append(acc * inv)
            outs[g] = o
            chain.append(o[NJ - 1])
            if g % 2 == 1:
                o0 = outs.pop(g - 1)
                o1 = outs.pop(g)
                pk = [pack2(o0[j], o1[j]) for j in range(NJ)]
                for j in range(NJ):
                    o_c[j, pl.ds(32 * (g // 8) + (g // 2) % 4, 8, stride=4), :] = pk[j]
                if FA:
                    fin(dl, orall(pk[NJ - FA:]))

        def emit(i, tk):
            if i < NG:
                a1(order[i], tk())
            if 0 <= i - 1 < NG:
                a2(order[i - 1])
            if 0 <= i - 2 < NG:
                a3(order[i - 2], slots[i - 2] + (WA if t < 5 else WA2 if t < 7 else WA3))
        return slots + [slots[-1] + 1, slots[-1] + 2], emit

    def st_halo(t, kv, slots):
        dst, src = BUF[t % 3][kv], BUF[(t - 1) % 3][kv]

        def emit(j, tk):
            sub = lax.broadcasted_iota(i32, (8, 128), 0) | pltpu.bitcast(tk(), i32)
            for m in range(1, HV + 1):
                a0 = (HV + NG - m) * 8
                if t == 0:
                    top = 0.0
                else:
                    top = src[j, a0 + 7:a0 + 15, :]
                    if t == 2 and kv == 2:
                        top = top + bias_v[NJ + j]
                dst[j, (HV - m) * 8:(HV - m + 1) * 8, :] = jnp.where(sub < 1, top, dst[j, a0 - 1:a0 + 7, :])
        return slots, emit

    def st_ln1(t, slots, fin, mo):
        h_r, row0 = BUF[t % 3][0], t * TM
        l1, hs = {}, {}
        order = [2 * (4 * i + m) + p for m in mo for i in range(4) for p in range(2)]

        def ldx(g, z):
            r = 64 * (g // 8) + 8 * ((g // 2) % 4) + 32 * (g % 2)
            return [x_3[z, pl.ds(row0 + r, 8), j * 128:(j + 1) * 128].astype(f32) for j in range(NJ)]

        def n1(g, tok):
            xf = ldx(g, 0)
            xf[0] = xf[0] + pltpu.bitcast(tok, f32)
            l1[g] = (lsum(tree(xf)), lsum(tree([x * x for x in xf])))

        def n3(g, dl):
            m, rs = stats(*l1.pop(g))
            xf = ldx(g, zs[0])
            hs[g] = [(xf[j] - m) * rs * mrow(1, j) for j in range(NJ)]
            if t > 1:
                hs[g] = [hs[g][j] + mrow(0, j) for j in range(NJ)]
            if g % 2 == 1:
                b = g // 2
                h0 = hs.pop(g - 1)
                h1 = hs.pop(g)
                pk = [pack2(h0[j], h1[j]) for j in range(NJ)]
                for j in range(NJ):
                    h_r[j, pl.ds(32 * (b % 4) + b // 4, 8, stride=4), :] = pk[j]
                if FL:
                    fin(dl, orall(pk[NJ - FL:]))

        def emit(i, tk):
            if i < NG:
                n1(order[i], tk())
            if 0 <= i - 1 < NG:
                n3(order[i - 1], slots[i - 1] + (WL if t > 1 else 20 if i < 12 else 8))
        return slots + [slots[-1] + 1], emit

    def st_apply(t, slots, fin):
        order = sorted(range(NG // 2), key=lambda b: b % 4)

        def emit(i, tk):
            b = order[i]
            r = t * TM + 64 * (b // 4) + 8 * (b % 4)
            pk = [pack2(h2_v[r:r + 8, j * 128:(j + 1) * 128] * mrow(1, j),
                        h2_v[r + 32:r + 40, j * 128:(j + 1) * 128] * mrow(1, j)) for j in range(NJ)]
            for j in range(NJ):
                BUF[t][0][j, pl.ds(32 * (b % 4) + b // 4, 8, stride=4), :] = pk[j]
            if fin is not None:
                fin(slots[i] + 3, orall(pk))
        return slots, emit

    def st_post(t, slots, fin, mo, snap=None):
        x1_rs, row0 = x1s[4 * (t % 2):4 * (t % 2) + 4], t * TM
        p1s, p3s, bst, ends = {}, {}, {}, []
        order = [4 * ci + m for m in mo for ci in range(GM)]

        def ldx1(g, z):
            return [x1_rs[g % 4][j, pl.ds((g // 4) * 8 + zo(z), 8), :] for j in range(NJ)]

        def p1(g, tok):
            xf = ldx1(g, 0)
            if tok is not None:
                xf[0] = xf[0] + pltpu.bitcast(tok, f32)
            p1s[g] = (lsum(tree(xf)), lsum(tree([x * x for x in xf])))

        def p3(g, dl):
            x1 = ldx1(g, 1)
            m, rs = stats(*p1s.pop(g))
            nn = [(x1[j] - m) * rs for j in range(NJ)]
            ov = [(x1[j] + mrow(7, j)) + nn[j] * mrow(6, j) for j in range(NJ)]
            p3s[g] = lsum(tree([nn[j] * mrow(8, j) for j in range(NJ)]))
            h2_v[pl.ds(row0 + g * 8, 8), :] = jnp.concatenate(nn, axis=1)
            out_v[pl.ds(row0 + g * 8, 8), :] = jnp.concatenate(ov, axis=1).astype(bf16)
            ends.append(orall([pltpu.bitcast(o, u32) for o in ov[PT:]]))
            fin(dl, ends[-1])

        def p4(g, n, dl):
            rg = (p3s.pop(g) + mrow(9, 0)).astype(bf16).astype(f32)
            m = g % 4
            if n % GM == 0:
                bst['v'] = best_v[m * 8:(m + 1) * 8, :]
                bst['i'] = besti_v[m * 8:(m + 1) * 8, :]
            upd = rg > bst['v']
            bst['v'] = jnp.where(upd, rg, bst['v'])
            bst['i'] = jnp.where(upd, row0 + g * 8, bst['i'])
            if n % GM == GM - 1:
                best_v[m * 8:(m + 1) * 8, :] = bst['v']
                besti_v[m * 8:(m + 1) * 8, :] = bst['i']
            if n % 2 == 1:
                fin(dl, pltpu.bitcast(bst['i'], u32))

        def emit(i, tk):
            if i < NG:
                p1(order[i], tk())
            if 0 <= i - 1 < NG:
                p3(order[i - 1], slots[i - 1] + WP)
            if 0 <= i - 2 < NG:
                p4(order[i - 2], i - 2, slots[i - 2] + WP + 2)
            if snap is not None and i - 2 == SNAP * GM - 1:
                snap()
            if t == NT - 1 and i == 2 * GM:
                [cp_.start() for cp_ in last_cp(mo[0] // 2)]
            if i == NG:
                [cp_.start() for cp_ in (last_cp(mo[2] // 2) if t == NT - 1 else [out_cp(t)])]
                if t == NT - 1:
                    spec.append(orall(ends[2 * GM:]))
        return slots + [slots[-1] + 1, slots[-1] + 2], emit

    def st_perm(t, js, slots, fin, dl, r0=0):
        cst = {}

        def emit(i_, tk):
            r = r0 + i_
            if i_ == 0:
                lane = lax.broadcasted_iota(i32, (8, 128), 1)
                cls = (lane // 4) % 5
                cst['m'] = [cls == c for c in range(1, NJ)]
                for j in js:
                    cst[j] = 4 * ((5 * (lane % 32) + j) % 32) + lane // 32
            srcs = [tou(wqkv_raw[r * 16:(r + 1) * 16, t * D + i * 128:t * D + (i + 1) * 128]) for i in range(NJ)]
            for j in js:
                m = srcs[(j * 3) % 5]
                if tk() is not None:
                    m = m | tk()
                for c in range(1, NJ):
                    m = jnp.where(cst['m'][c - 1], srcs[((j + 5 - c) * 3) % 5], m)
                m = jnp.take_along_axis(m, cst[j], axis=1)
                wq_p[t * NJ + j][r * 8:(r + 1) * 8, :] = m
            if fin is not None:
                fin(slots[i_] + dl, m)
        return slots, emit

    def st_perm_o(slots, fin, dl):
        def emit(i, tk):
            n, j = (i % 25) // NJ, i % NJ
            if i < 25:
                w = wo_raw[j * 128:(j + 1) * 128, n * 128:(n + 1) * 128].astype(f32) * (
                    mrow(2, n) + pltpu.bitcast(tk(), f32))[0:1]
                wo_f[n, j * 128:(j + 1) * 128, :] = w
                fin(slots[i] + dl, pltpu.bitcast(w[120:128], u32))
                return
            for dd in range(4):
                for hh in range(2):
                    r0 = hh * 16 * DH + 4 * j + dd
                    ev = wo_f[n, pl.ds(r0, 8, stride=2 * DH), :]
                    od = wo_f[n, pl.ds(r0 + DH, 8, stride=2 * DH), :]
                    p0 = j * 64 + dd * 16 + hh * 8
                    pk = pack2(ev, od)
                    wo_p[n][p0:p0 + 8, :] = pk
            fin(slots[i] + dl, pk)
        return slots, emit

    class Phase:
        def __init__(self, carry=None):
            self.done = {}
            self.tok = None
            if carry is not None:
                self.done = dict(carry.left)
                self.tok = carry.tok
            self.cur = 0

        def fin(self, slot, v):
            self.done.setdefault(max(slot, self.cur), []).append(v)

        def run(self, jobs, streams):
            pos = [0] * len(streams)
            pend = []
            for c in range(len(jobs) + 1):
                self.cur = c
                cache = []

                def tk():
                    if self.tok is None:
                        return None
                    if not cache:
                        cache.append(zand(self.tok))
                    return cache[0]
                for si, (slots, emit) in enumerate(streams):
                    while pos[si] < len(slots) and (slots[pos[si]] <= c or c == len(jobs)):
                        emit(pos[si], tk)
                        pos[si] += 1
                if c == len(jobs):
                    break
                pend += self.done.pop(c, [])
                r = jobs[c](pend)
                if r is not None:
                    self.tok = r
                    pend = []
            self.left = {k - len(jobs): v for k, v in self.done.items()}

    def out_cp(t):
        return pltpu.make_async_copy(out_v.at[pl.ds(t * TM, TM)], out_hbm.at[pl.ds(t * TM, TM)],
                                     sems.at[1 if t <= ST else NSEM])

    def last_cp(h):
        rs = [(NT - 1) * TM + 32 * ci + 16 * h for ci in range(GM)]
        return [pltpu.make_async_copy(out_v.at[pl.ds(r, 16)], out_hbm.at[pl.ds(r, 16)], sems.at[NSEM]) for r in rs]

    def wait_late():
        for cp_ in [out_cp(t) for t in range(ST + 1, NT - 1)] + last_cp(0) + last_cp(1):
            cp_.wait()

    best_v[...] = jnp.full((32, 128), -jnp.inf, f32)
    besti_v[...] = jnp.zeros((32, 128), i32)
    for r_ in (ka, kb, kc, va, vb, vc):
        for j in range(NJ):
            r_[j, KVR - 8:KVR, :] = jnp.zeros((8, 128), f32)
    wait(g_z)
    zv = pltpu.bitcast(zero_v[...], i32)
    for i in range(4):
        zs[i] = zv[i, 0]
    wait(g_x0)
    cf = c_v[...].astype(f32)
    sc_v[...] = tou(jnp.broadcast_to((cf * jax.nn.sigmoid(cf)).astype(bf16), (16, D)))
    for g in range(NG):
        xf = [x_v[g * 8:(g + 1) * 8, j * 128:(j + 1) * 128].astype(f32) for j in range(NJ)]
        m_, rs_ = stats(lsum(tree(xf)), lsum(tree([x * x for x in xf])))
        h2_v[g * 8:(g + 1) * 8, :] = jnp.concatenate([(x - m_) * rs_ for x in xf], axis=1)
    wait(g_ca)
    for j in range(NJ):
        job_mod(1, j)([])
    Phase().run([], [st_apply(0, [0] * 16, None)])
    wait(g_wq)

    ph = Phase()
    fin = ph.fin
    mo = [2, 3, 0, 1]
    nat = list(range(NM))
    jobs, streams, spec = [], [], []

    def nmaj(t, ns, bias=False):
        return [job_qkv(t, n, m, (1 if m == 0 else 2) if bias == 1 else bias) for n in ns for m in nat]

    def mmaj(t, ns):
        return [job_qkv(t, n, m) for m in mo for n in ns]

    def waiter(g, *keys):
        def f():
            wait(g)
        return job_call(f)

    QS, KS, VS = range(NJ), range(NJ, 2 * NJ), range(2 * NJ, 3 * NJ)
    K3 = 52; K5 = 6; K4 = 2
    K1 = 18
    KX = 20; PH = 1; PL = 0; L0 = 36
    jobs += [job_q0(n, m, hi) for hi in range(2) for n in QS for m in nat]
    jobs += mmaj(1, QS) + nmaj(0, KS) + nmaj(1, KS)[:KX]
    jobs.insert(80 + KX - K5, waiter(g_wv, ('raw', 2), 'x2'))
    for j in range(NJ):
        jobs.insert(80 + KX - K5 + 1 + [j, 2 * j, (3 * j) // 2, 2 * j + 1][1], job_mod(0, j))
    jobs.insert(K1, waiter(g_wq2, 'x1'))
    jobs.insert(K3, waiter(g_wk, ('raw', 1)))
    s5 = 83 + KX - K5
    sv0 = len(jobs)
    for j in range(NJ):
        jobs += nmaj(0, [2 * NJ + j], 1) + [job_bq(j)]
    sk1 = len(jobs)
    jobs += nmaj(1, KS)[KX:]
    sv1 = len(jobs)
    for j in range(NJ):
        jobs += nmaj(1, [2 * NJ + j], 2) + [job_bq(NJ + j)]
    jobs.insert(len(jobs) - K4, waiter(g_xr, 'x'))
    s4 = len(jobs) - K4
    for j in range(NJ):
        streams.append(st_perm(0, [j], [[0, 0, PL, 1, 3][j]] * QLO, None, 0))
        streams.append(st_perm(0, [j], [K1 + [1, 1, 1, 1 + PH, 1 + 3 * PH][j]] * (40 - QLO), None, 0, QLO))
    streams.append(st_ln1(1, _spread(12, K1 + 1, L0) + _spread(NG - 12, L0, 48), fin, mo))
    PK = 4; PV = 10
    streams += [st_perm(1, [j], _spread(40, K3 + 1 + PK * j, K3 + 1 + PK * (j + 1)), None, 0) for j in range(NJ)]
    streams += [st_perm(2, [j], _spread(40, max(s5, sv0 + 5 * j - PV), max(s5 + 1, sv0 + 5 * j - PV + 5)), None, 0)
                for j in range(NJ)]
    st = {}
    for t in range(2, NT):
        if t == 6:
            jobs.append(waiter(g_rest))
        st[t] = len(jobs)
        jl = mmaj(t, QS) + nmaj(t, KS) + nmaj(t, VS) if t < NT - 1 else mmaj(t, KS) + nmaj(t, VS) + mmaj(t, QS)
        for i, jb in enumerate(jl):
            jobs.append(jb)
            if t == 6 and i % 3 == 1:
                jobs.append(job_mod(2 + (i // 3) // NJ, (i // 3) % NJ))

    def consts():
        cb, sb, gbv = mod_v[:, 4 * D:5 * D], mod_v[:, 3 * D:4 * D], mod_v[:, 5 * D:6 * D]
        wr = jnp.broadcast_to(wr_v[...].astype(f32).reshape(1, D), (8, D))
        mod_v[:, 6 * D:7 * D] = gbv * cb
        mod_v[:, 7 * D:8 * D] = gbv * sb
        mod_v[:, 8 * D:9 * D] = cb * wr
        mod_v[:, 9 * D:9 * D + 128] = jnp.broadcast_to(lsum(sb * wr), (8, 128))

    jobs.insert(st[7] + 20, job_call(consts))
    f6, f7 = st[7], len(jobs)

    def argmax(row):
        bv = best_v[...]
        bi = besti_v[...] + (lax.broadcasted_iota(i32, (32, 128), 0) & 7)
        mx = jnp.max(bv, axis=0, keepdims=True)
        cand = jnp.where(bv == mx, bi, S)
        idxv = jnp.min(cand, axis=0, keepdims=True)
        idx = jnp.minimum(idxv, ((ST + 1) * TM if row else S) - 1)[0, 0]
        return mx, idx, h2_v[pl.ds(idx, 1), :] if row else None

    def glu(g, u):
        hg = 0.5 * g
        return (hg * jnp.tanh(hg) + hg) * u

    def wrow(w_v, r0, j):
        return w_v[r0:r0 + 8, j * 128:(j + 1) * 128].astype(f32)

    def moe_in(nrow):
        hrow = jnp.broadcast_to(nrow, (8, D)) * mod_v[:, 4 * D:5 * D] + mod_v[:, 3 * D:4 * D]
        hrow = hrow.astype(bf16).astype(f32)
        return [hrow[:, j * 128:(j + 1) * 128] for j in range(NJ)]

    def vgroup(r0, h0, acc):
        g = lsum(tree([wrow(wg_v, r0, j) * h0[j] for j in range(NJ)]))
        u = lsum(tree([wrow(wu_v, r0, j) * h0[j] for j in range(NJ)]))
        av = glu(g, u)
        pr = [wrow(wd_v, r0, j) * av for j in range(NJ)]
        return pr if acc is None else [acc[j] + pr[j] for j in range(NJ)]

    early = {'acc': None}

    def st_moe(slots, fin):
        def emit(i, tk):
            if i == 0:
                early['hf'] = moe_in(spec[0][2])
            hf = early['hf']
            h0 = [hf[0] + pltpu.bitcast(tk(), f32)] + hf[1:]
            for k in (2 * i, 2 * i + 1):
                early['acc'] = vgroup(NC * 128 + k * 8, h0, early['acc'])
            fin(slots[i] + WM, orall([pltpu.bitcast(a, u32) for a in early['acc'][3:]]))
        return slots, emit

    def gap(n, lo, hi, bar, taper):
        return [x if x < bar - taper else x + taper + 1 for x in _spread(n, lo, hi - taper - 1)]

    TP = 5; AX = 22; AY = 4; LX = -10
    streams += [st_halo(0, 2, _spread(NJ, sv0 + 4, sv0 + 20)), st_halo(0, 3, _spread(NJ, sk1 + 4, sk1 + 14)),
                st_halo(1, 2, _spread(NJ, sv1 + 4, sv1 + 14)), st_halo(1, 3, _spread(NJ, st[2] + 4, st[2] + 16))]
    for t in range(2, NT - 1):
        streams += [st_halo(t, 2, _spread(NJ, st[t + 1] - 16, st[t + 1] - 6)),
                    st_halo(t, 3, _spread(NJ, st[t + 1] + 4, st[t + 1] + 16))]
    streams += [st_halo(7, 2, _spread(NJ, f6 + 28, f6 + 42)), st_halo(7, 3, _spread(NJ, f6 + 48, f6 + 60))]
    a_lo = [sk1 + 2, st[2] + AX, st[3] + AX - AY, st[4] + AX - 2 * AY, st[5] + max(AX - 3 * AY, 1)]
    streams.append(st_attention(0, gap(NG, a_lo[0], a_lo[1], s4 - 1, TP), fin))
    for t in range(1, 4):
        streams.append(st_attention(t, _spread(NG, a_lo[t], a_lo[t + 1]), fin))
    A5 = 4
    streams.append(st_attention(4, gap(NG, a_lo[4], st[6] + A5, st[6] - 1, ATHI - 1), fin))
    T0 = 0; T1 = 46; T2 = 46; T3 = 94; T4 = 10; T5 = 6
    streams.append(st_attention(5, _spread(NG, st[6] + A5, f6 + T0), fin))
    streams.append(st_attention(6, _spread(NG, f6 + max(T0, 1), f6 + T1), fin))
    streams.append(st_attention(7, _spread(T4, f6 + T2, f7 + T5) + _spread(NG - T4, f7 + T5, f7 + T3), fin,
                                order=[(i + 16) % NG for i in range(NG)]))
    streams.append(st_ln1(2, _spread(NG, s5 + 10, sk1 + 4), fin, mo))
    for t in range(3, 6):
        streams.append(st_ln1(t, _spread(NG, max(st[t - 1] + LX, s4), st[t] + LX), fin, mo))
    streams.append(st_ln1(6, _spread(NG, st[5] + LX, st[6] - LNHI), fin, mo))
    streams.append(st_ln1(7, _spread(NG, st[6], st[7] + 0), fin, mo))
    streams.append(st_perm_o(_spread(25, f6 + 4, f6 + 24) + _spread(25, f6 + 24 + 2, f6 + 54),
                             fin, 4))
    for t in range(NT):
        mt = mo if t == NT - 1 else nat
        jobs += [job_wo(t, c, m) for m in mt for c in range(NJ)]
        s0 = f7 + 20 * t + POLO
        sl = _spread(NG, s0, s0 + 20)
        if t == NT - 1:
            sl = [min(sl[i], s0 - POLO + PL7 + 5 * (i // 8) + (i % 8) // 3) for i in range(NG)]
        streams.append(st_post(t, sl, fin, mt,
                               (lambda: spec.append(argmax(True))) if t == ST else None))
    m0 = f7 + 20 * ST + POLO + 5 * SNAP + 2
    streams.append(st_moe(_spread(NE // 2, m0, f7 + 160 + 0), fin))
    ph.run(jobs, streams)

    def moe(mx, idx, hf, NC, n0, acc, after=None):
        base = pl.multiple_of((idx // 16) * 16, 16)
        h16 = [tob(pack2(h, h)) for h in hf]
        NV = (F - NC * 128) // 8 - n0

        def ntdot(w_v, c):
            return tree([lax.dot_general(h16[j], w_v[c * 128:(c + 1) * 128, j * 128:(j + 1) * 128],
                                         (((1,), (1,)), ((), ())),
                                         preferred_element_type=f32)[0:8] for j in range(NJ)])

        ym, acts, toks = None, [], []
        MD = 2
        MA = 2
        NP = 2 * NC - 1 + MD
        for c in range(2 * NC + 2):
            if c < 2 * NC:
                toks.append(ntdot(wu_v if c % 2 else wg_v, c // 2))
                if c % 2:
                    a8 = glu(toks[c - 1], toks[c])
                    acts.append(tob(pack2(a8, a8)))
            if c > 2 and c % 2:
                k = (c - 3) // 2
                yc = [jnp.dot(acts[k], wd_v[k * 128:(k + 1) * 128, j * 128:(j + 1) * 128],
                              preferred_element_type=f32)[0:8] for j in range(NJ)]
                ym = yc if ym is None else [ym[j] + yc[j] for j in range(NJ)]
            if c < NP:
                tk_ = None if c < MD else pltpu.bitcast(toks[c - MD], u32)
                if after is not None and c == MA:
                    tk_ = after if tk_ is None else tk_ | after
                h0 = hf if tk_ is None else [h + pltpu.bitcast(zand(tk_), f32) for h in hf]
                for i in range(c * NV // NP, (c + 1) * NV // NP):
                    acc = vgroup(NC * 128 + (n0 + i) * 8, h0, acc)
        y = jnp.concatenate(ym, axis=1)[0:1] + jnp.sum(jnp.concatenate(acc, axis=1), axis=0, keepdims=True)
        y = y * jax.nn.sigmoid(mx[:, 0:1])
        rows = base + lax.broadcasted_iota(i32, (16, D), 0)
        gb = mod_v[0:1, 5 * D:6 * D]
        old = out_v[pl.ds(base, 16), :].astype(f32)
        newblk = jnp.where(rows == idx, old + gb * y, old)
        fix_v[...] = newblk.astype(bf16)

    moe(spec[0][0], spec[0][1], early['hf'], NC, NE, early['acc'], spec[1])
    mx_f, idx_f, _ = argmax(False)
    idx_s = spec[0][1]
    for t in range(ST + 1):
        out_cp(t).wait()

    def fix(idx):
        base = pl.multiple_of((idx // 16) * 16, 16)
        return pltpu.make_async_copy(fix_v, out_hbm.at[pl.ds(base, 16)], sems.at[0])

    @pl.when(idx_f == idx_s)
    def _():
        fix(idx_s).start()
        wait_late()
        fix(idx_s).wait()

    @pl.when(idx_f != idx_s)
    def _():
        moe(mx_f, idx_f, moe_in(h2_v[pl.ds(idx_f, 1), :]), 7, 0, None)
        wait_late()
        fix(idx_f).start()
        fix(idx_f).wait()


@jax.jit
def pallas_adaLN_cond__sliding_local_dilated__moe_arch_mod__prompt_kernel(
    A_x, A_wqkv, A_wo, B_x, B_w_r, B_w_gate, B_w_up, B_w_down, c, w_mod,
):
    x = A_x.reshape(S, D)
    V = pltpu.VMEM
    scratch = [V((D // 2, 128), u32)] * 20 + [V((NJ, MS, 128), f32)] * 8 + [
        V((1, S, D), bf16),
        V((3 * NJ + 1, 8, 128), f32),
        V((D, 3 * D), bf16),
        V((D, D), bf16),
        V((NJ, D, 128), f32),
        V((F, D), bf16),
        V((F, D), bf16),
        V((F, D), bf16),
        V((D, 6 * D), bf16),
        V((8, 9 * D + 128), f32),
        V((NJ, TM // 2, 128), u32), V((NJ, TM // 2, 128), u32), V((NJ, TM // 2, 128), u32),
        V((NJ, TM, 128), f32), V((NJ, TM, 128), f32), V((NJ, TM, 128), f32),
        V((NJ, KVR, 128), f32), V((NJ, KVR, 128), f32), V((NJ, KVR, 128), f32),
        V((NJ, KVR, 128), f32), V((NJ, KVR, 128), f32), V((NJ, KVR, 128), f32),
        V((NT - 1, NJ, TM // 2, 128), u32), V((NJ, TM // 2, 128), u32),
        V((S, D), f32),
        V((S, D), bf16),
        V((32, 128), f32),
        V((32, 128), i32),
        V((8, 128), u32),
        V((8, 128), u32),
        V((8, D), u32),
        V((8, D), u32),
        V((16, D), bf16),
        V((1, D), bf16),
        V((D,), bf16),
        pltpu.SMEM((4,), i32),
        pltpu.SemaphoreType.DMA((NSEM + 1,)),
    ]
    out = pl.pallas_call(
        _kernel,
        out_shape=jax.ShapeDtypeStruct((S, D), bf16),
        in_specs=[pl.BlockSpec(memory_space=pltpu.HBM)] * 9,
        out_specs=pl.BlockSpec(memory_space=pltpu.HBM),
        scratch_shapes=scratch,
        compiler_params=pltpu.CompilerParams(vmem_limit_bytes=100 * 2**20),
    )(x, A_wqkv, A_wo, B_w_r, B_w_gate.T, B_w_up.T, B_w_down, c, w_mod)
    return out.reshape(1, S, D)
```
